```python
import os as _os
_os.environ.setdefault("JAX_PLATFORMS", "cpu")
import jax
import jax.numpy as jnp

def _softmax(x, axis=-1):
    return jax.nn.softmax(x, axis=axis)
def _gelu(x):
    return jax.nn.gelu(x, approximate=True)
def _silu(x):
    return jax.nn.silu(x)
def _sigmoid(x):
    return jax.nn.sigmoid(x)
def _layernorm(x, axis=-1, eps=1e-5):
    m = jnp.mean(x, axis=axis, keepdims=True)
    v = jnp.var(x, axis=axis, keepdims=True)
    return (x - m) / jnp.sqrt(v + eps)
def _scatter_add(tgt, idx, src, axis=0):
    return tgt.at[idx].add(src)
def _segment_sum(src, seg, n):
    return jax.ops.segment_sum(src, seg, n)
class _Rng:
    def __init__(self, key):
        self._k = key
    def _next(self):
        self._k, sub = jax.random.split(self._k)
        return sub
    def normal(self, shape):
        return jax.random.normal(self._next(), shape, dtype=jnp.bfloat16)
    def randint(self, lo, hi, shape):
        return jax.random.randint(self._next(), shape, lo, hi, dtype=jnp.int32)
    def uniform(self, shape, lo=0.0, hi=1.0):
        return jax.random.uniform(self._next(), shape, jnp.bfloat16, lo, hi)
    def permutation(self, n):
        return jax.random.permutation(self._next(), n)


kernel_name = 'sequential_preLN__softmax_full_mha__dense_activation_squared_relu__prompt'

def setup_inputs():
    _rng = _Rng(jax.random.key(int.from_bytes(__import__("os").urandom(4), "little")))
    _w = (lambda a: (lambda t: t.astype(jnp.bfloat16) if jnp.issubdtype(t.dtype, jnp.floating) else t)(jnp.asarray(a)))
    def _A_setup():
        B, S, D = 1, 2048, 448
        return {
            "x": _w((lambda *s: _rng.normal(s) * 0.05)(B, S, D)),
            "wqkv": _w((lambda *s: _rng.normal(s) * 0.05)(D, 3 * D)),
            "wo": _w((lambda *s: _rng.normal(s) * 0.05)(D, D)),
        }
    _A_in = _A_setup()

    def _B_setup():
        B, S, D, F = 1, 2048, 448, 1792
        return {
            "x": _w((lambda *s: _rng.normal(s) * 0.05)(B, S, D)),
            "w1": _w((lambda *s: _rng.normal(s) * 0.05)(D, F)),
            "b1": _w((lambda *s: _rng.normal(s) * 0.05)(F)),
            "w2": _w((lambda *s: _rng.normal(s) * 0.05)(F, D)),
            "b2": _w((lambda *s: _rng.normal(s) * 0.05)(D)),
        }
    _B_in = _B_setup()

    return {
        "A_x": _A_in["x"],
        "A_wqkv": _A_in["wqkv"],
        "A_wo": _A_in["wo"],
        "B_x": _B_in["x"],
        "B_w1": _B_in["w1"],
        "B_b1": _B_in["b1"],
        "B_w2": _B_in["w2"],
        "B_b2": _B_in["b2"],
    }

def reference(A_x, A_wqkv, A_wo, B_x, B_w1, B_b1, B_w2, B_b2):
    def _A_ref(x, wqkv, wo):
        B, S, D = x.shape
        H = 16; Dh = D // H
        qkv = (lambda x, *d: x.transpose(*d))((x @ wqkv).reshape(B, S, 3, H, Dh), 2, 0, 3, 1, 4)
        q, k, v = qkv[0], qkv[1], qkv[2]
        scale = Dh ** -0.5
        scores = jnp.einsum("bhqd,bhkd->bhqk", q, k) * scale
        p = _softmax(scores, axis=-1)
        o = jnp.einsum("bhqk,bhkd->bhqd", p, v)
        return (lambda x, *d: x.transpose(*d))(o, 0, 2, 1, 3).reshape(B, S, D) @ wo

    def _B_ref(x, w1, b1, w2, b2):
        h = jnp.einsum("bsd,df->bsf", x, w1) + b1
        zero = jnp.zeros_like(h)
        r = jnp.where(h > zero, h, zero)
        h = r * r
        out = jnp.einsum("bsf,fd->bsd", h, w2) + b2
        return out

    x = A_x
    h = x + _A_ref(_layernorm(x, axis=-1), A_wqkv, A_wo)
    h2 = h + _B_ref(_layernorm(h, axis=-1), B_w1, B_b1, B_w2, B_b2)
    return h2
```

```python
import math

import jax
import jax.numpy as jnp
import jax.experimental.pallas as pl
import jax.experimental.pallas.tpu as pltpu

H = 16
HP = 32
HG = 4
EPS = 1e-5
TR = 512
TQ = 512
CK = 128

_NT = (((1,), (1,)), ((), ()))


def _layernorm(x):
    m = jnp.mean(x, axis=-1, keepdims=True)
    xc = x - m
    v = jnp.mean(xc * xc, axis=-1, keepdims=True)
    return xc * jax.lax.rsqrt(v + EPS)


def _kernel(x_ref, wqkv_ref, wo_ref, w1_ref, b1_ref, w2_ref, b2_ref, out_ref,
            wqk_s, wvt_s, wot_s, k_s, q_s, vt_s, ot_s, s_s, m_s):
    S, D = x_ref.shape
    DH = D // H
    GW = HG * DH
    NG = H // HG
    NJ = S // TQ
    NC = S // CK
    f32, bf16 = jnp.float32, jnp.bfloat16
    qscale = (DH ** -0.5) * math.log2(math.e)

    for g in range(NG):
        wqk_s[:, g * 128:(g + 1) * 128] = wqkv_ref[:, g * GW:g * GW + 128]
        wqk_s[:, (NG + g) * 128:(NG + g + 1) * 128] = wqkv_ref[:, D + g * GW:D + g * GW + 128]
    wvt = wqkv_ref[:, 2 * D:3 * D].astype(f32).T
    wo = wo_ref[...].astype(f32)
    zpad = jnp.zeros((HP - DH, D), f32)
    wvt_p = jnp.concatenate(
        [t for h in range(H) for t in (wvt[h * DH:(h + 1) * DH], zpad)], axis=0)
    wo_p = jnp.concatenate(
        [t for h in range(H) for t in (wo[h * DH:(h + 1) * DH], zpad)], axis=0)
    wvt_s[...] = wvt_p.astype(bf16)
    wot_s[...] = wo_p.T.astype(bf16)

    lane = jax.lax.broadcasted_iota(jnp.int32, (TR, 128), 1)
    vrow = jax.lax.broadcasted_iota(jnp.int32, (H * HP, TR), 0)
    ones_row = (vrow % HP) == DH
    for r in range(S // TR):
        rows = pl.ds(r * TR, TR)
        xn = _layernorm(x_ref[rows, :].astype(f32)).astype(bf16)
        qk = jnp.dot(xn, wqk_s[...], preferred_element_type=f32)
        for g in range(NG):
            qg = qk[:, g * 128:(g + 1) * 128] * qscale
            for i in range(HG):
                msk = (lane >= i * DH) & (lane < (i + 1) * DH)
                q_s[g * HG + i, rows, :] = jnp.where(msk, qg, 0.0).astype(bf16)
            k_s[g, rows, :] = qk[:, (NG + g) * 128:(NG + g + 1) * 128].astype(bf16)
        vt = jax.lax.dot_general(wvt_s[...], xn, _NT, preferred_element_type=f32)
        vt = jnp.where(ones_row, 1.0, vt).astype(bf16)
        vt_s[:, :, rows] = vt.reshape(H, HP, TR)

    def qk_chunk(h, j, c, m):
        q = q_s[h, pl.ds(j * TQ, TQ), :]
        k = k_s[h // HG, pl.ds(c * CK, CK), :]
        s = jax.lax.dot_general(k, q, _NT, preferred_element_type=f32)
        s_s[j, pl.ds(c * CK, CK), :] = s
        mc = jnp.max(s.reshape(CK // 8, 8, TQ), axis=0)
        return mc if m is None else jnp.maximum(m, mc)

    def pv_chunk(h, j, c, m, acc):
        s = s_s[j, pl.ds(c * CK, CK), :]
        p = jnp.exp2(s - m).astype(bf16)
        vt = vt_s[h, :, pl.ds(c * CK, CK)]
        o = jnp.dot(vt, p, preferred_element_type=f32)
        return o if acc is None else acc + o

    def pv_finish(h, j, acc):
        l = acc[DH:DH + 1, :]
        ot_s[h, :, pl.ds(j * TQ, TQ)] = (acc / l).astype(bf16)

    for j in range(NJ):
        m = None
        for c in range(NC):
            m = qk_chunk(0, j, c, m)
        m_s[j] = jnp.max(m, axis=0, keepdims=True)

    def body(h, carry):
        for j in range(NJ):
            mcur = m_s[j]
            m = None
            acc = None
            for c in range(NC):
                acc = pv_chunk(h, j, c, mcur, acc)
                m = qk_chunk(h + 1, j, c, m)
            pv_finish(h, j, acc)
            m_s[j] = jnp.max(m, axis=0, keepdims=True)
        return carry

    jax.lax.fori_loop(0, H - 1, body, 0)

    for j in range(NJ):
        mcur = m_s[j]
        acc = None
        for c in range(NC):
            acc = pv_chunk(H - 1, j, c, mcur, acc)
        pv_finish(H - 1, j, acc)

    b1 = b1_ref[...].astype(f32)
    b2 = b2_ref[...].astype(f32)
    for r in range(S // TR):
        rows = pl.ds(r * TR, TR)
        ot = ot_s[:, :, rows].reshape(H * HP, TR)
        attn_t = jnp.dot(wot_s[...], ot, preferred_element_type=f32)
        h1 = x_ref[rows, :].astype(f32) + attn_t.T
        xn2 = _layernorm(h1).astype(bf16)
        hid = jnp.dot(xn2, w1_ref[...], preferred_element_type=f32) + b1
        hid = jnp.maximum(hid, 0.0)
        hid = (hid * hid).astype(bf16)
        y = jnp.dot(hid, w2_ref[...], preferred_element_type=f32) + b2
        out_ref[rows, :] = (h1 + y).astype(out_ref.dtype)


@jax.jit
def pallas_sequential_preLN__softmax_full_mha__dense_activation_squared_relu__prompt_kernel(
    A_x: jax.Array,
    A_wqkv: jax.Array,
    A_wo: jax.Array,
    B_x: jax.Array,
    B_w1: jax.Array,
    B_b1: jax.Array,
    B_w2: jax.Array,
    B_b2: jax.Array,
):
    del B_x
    B, S, D = A_x.shape
    F = B_w1.shape[1]
    assert B == 1
    bf16 = jnp.bfloat16
    out = pl.pallas_call(
        _kernel,
        out_shape=jax.ShapeDtypeStruct((S, D), A_x.dtype),
        scratch_shapes=[
            pltpu.VMEM((D, 2 * (H // HG) * 128), bf16),
            pltpu.VMEM((H * HP, D), bf16),
            pltpu.VMEM((D, H * HP), bf16),
            pltpu.VMEM((H // HG, S, 128), bf16),
            pltpu.VMEM((H, S, 128), bf16),
            pltpu.VMEM((H, HP, S), bf16),
            pltpu.VMEM((H, HP, S), bf16),
            pltpu.VMEM((S // TQ, S, TQ), jnp.float32),
            pltpu.VMEM((S // TQ, 1, TQ), jnp.float32),
        ],
        compiler_params=pltpu.CompilerParams(vmem_limit_bytes=100 * 2**20),
    )(A_x.reshape(S, D), A_wqkv, A_wo, B_w1, B_b1.reshape(1, F), B_w2, B_b2.reshape(1, D))
    return out.reshape(B, S, D)
```

```python
import math

import jax
import jax.numpy as jnp
import jax.experimental.pallas as pl
import jax.experimental.pallas.tpu as pltpu

H = 16
HP = 32
HG = 4
EPS = 1e-5
TR = 512
TQ = 512
CK = 128
DA = 16

f32, bf16, u32 = jnp.float32, jnp.bfloat16, jnp.uint32


def _pk(x):
    return pltpu.bitcast(x, u32)


def _up(x):
    return pltpu.bitcast(x, bf16)


def _layernorm_t(x):
    m = jnp.mean(x, axis=0, keepdims=True)
    xc = x - m
    v = jnp.mean(xc * xc, axis=0, keepdims=True)
    return xc * jax.lax.rsqrt(v + EPS)


def _kernel(xt_hbm, wqkv_hbm, wo_hbm, w1_hbm, b1_hbm, w2t_hbm, b2_hbm, out_hbm,
            xt_ref, wqkv_ref, wo_ref, w1_ref, b1_ref, w2t_ref, b2_ref, out_ref, sems,
            wt_s, wot_s, w1t_s, w2t_s, b2c_s, k_s, qt_s, vt_s, ot_s, s_s, m_s):
    D, S = xt_ref.shape
    F = w1_ref.shape[1]
    DH = D // H
    PAD = HP - DH
    GW = HG * DH
    NG = H // HG
    NJ = S // TQ
    NC = S // CK
    NR = S // TR
    qscale = (DH ** -0.5) * math.log2(math.e)

    def win(h):
        return h * DH - (PAD if h % 2 else 0)

    x0_copy = pltpu.make_async_copy(xt_hbm.at[:, 0:TR], xt_ref.at[:, 0:TR], sems.at[0])
    x1_copy = pltpu.make_async_copy(xt_hbm.at[:, TR:S], xt_ref.at[:, TR:S], sems.at[1])
    wqkv_copy = pltpu.make_async_copy(wqkv_hbm, wqkv_ref, sems.at[2])
    late_copies = [
        pltpu.make_async_copy(src, dst, sems.at[3 + i])
        for i, (src, dst) in enumerate([(wo_hbm, wo_ref), (w1_hbm, w1_ref), (b1_hbm, b1_ref),
                                        (b2_hbm, b2_ref), (w2t_hbm, w2t_ref)])]

    def out_copy(r):
        cols = pl.ds(r * TR, TR)
        return pltpu.make_async_copy(out_ref.at[:, cols], out_hbm.at[:, cols], sems.at[8 + r])

    def ln1(r):
        return _layernorm_t(xt_ref[:, pl.ds(r * TR, TR)].astype(f32)).astype(bf16)

    x0_copy.start()
    wqkv_copy.start()
    x0_copy.wait()
    xn_next = ln1(0)
    wqkv_copy.wait()
    x1_copy.start()

    wt_s[...] = _pk(wqkv_ref[...].T)
    grow = jax.lax.broadcasted_iota(jnp.int32, (GW, TR), 0)
    hrow = jax.lax.broadcasted_iota(jnp.int32, (HP, TR), 0)
    fill_even = jnp.where(hrow == DH, 1.0, 0.0)
    fill_odd = jnp.where(hrow == 0, 1.0, 0.0)
    zg = jnp.zeros((128 - GW, TR), bf16)
    for r in range(NR):
        cols = pl.ds(r * TR, TR)
        xn = xn_next
        if r == 1:
            pass
        qkvt = jnp.dot(_up(wt_s[...]), xn, preferred_element_type=f32)
        if r == 0:
            x1_copy.wait()
            for cp in late_copies:
                cp.start()
        if r + 1 < NR:
            xn_next = ln1(r + 1)
        for g in range(NG):
            qg = qkvt[g * GW:(g + 1) * GW] * qscale
            for i in range(HG):
                msk = (grow >= i * DH) & (grow < (i + 1) * DH)
                qm = jnp.where(msk, qg, 0.0).astype(bf16)
                qt_s[g * HG + i, :, cols] = _pk(jnp.concatenate([qm, zg], axis=0))
            kg = qkvt[D + g * GW:D + (g + 1) * GW].astype(bf16)
            k_s[g, pl.ds(r * TR // 2, TR // 2), :] = _pk(jnp.concatenate([kg, zg], axis=0).T)
        for h in range(H):
            vw = qkvt[2 * D + win(h):2 * D + win(h) + HP]
            if h % 2 == 0:
                vw = jnp.where(hrow < DH, vw, fill_even)
            else:
                vw = jnp.where(hrow >= PAD, vw, fill_odd)
            vt_s[h, :, cols] = _pk(vw.astype(bf16))

    def qk_chunk(h, j, c, m):
        qt = _up(qt_s[h, :, pl.ds(j * TQ, TQ)])
        k = _up(k_s[h // HG, pl.ds(c * CK // 2, CK // 2), :])
        s = jnp.dot(k, qt, preferred_element_type=f32)
        s_s[j, pl.ds(c * CK, CK), :] = s
        mc = jnp.max(s.reshape(CK // 8, 8, TQ), axis=0)
        return mc if m is None else jnp.maximum(m, mc)

    def pv_chunk(h, j, c, m, acc):
        s = s_s[j, pl.ds(c * CK, CK), :]
        p = jnp.exp2(s - m).astype(bf16)
        vt = _up(vt_s[h, :, pl.ds(c * CK, CK)])
        o = jnp.dot(vt, p, preferred_element_type=f32)
        return o if acc is None else acc + o

    def pv_finish(h, j, acc):
        l = jnp.where(h % 2 == 0, acc[DH:DH + 1, :], acc[0:1, :])
        ot_s[h, :, pl.ds(j * TQ, TQ)] = _pk((acc / l).astype(bf16))

    for cp in late_copies:
        cp.wait()
    wo = wo_ref[...].astype(f32)
    wrow = jax.lax.broadcasted_iota(jnp.int32, (HP, D), 0)
    wo_p = jnp.concatenate(
        [jnp.where((wrow < DH) if h % 2 == 0 else (wrow >= PAD),
                   wo[win(h):win(h) + HP], 0.0) for h in range(H)], axis=0)
    wot_s[...] = _pk(wo_p.T.astype(bf16))
    b1 = b1_ref[...].astype(f32)
    arow = jax.lax.broadcasted_iota(jnp.int32, (DA, 128), 0)
    for t in range(F // 128):
        aug = jnp.where(arow == 0, b1[t:t + 1, :], 0.0).astype(bf16)
        w1a = jnp.concatenate([w1_ref[:, t * 128:(t + 1) * 128], aug], axis=0)
        w1t_s[t * 64:(t + 1) * 64, :] = _pk(w1a.T)
    w2t_s[...] = _pk(w2t_ref[...])
    b2c_s[...] = jnp.broadcast_to(b2_ref[...].astype(f32), (128, D)).T

    for j in range(NJ):
        m = None
        for c in range(NC):
            m = qk_chunk(0, j, c, m)
        m_s[j] = jnp.max(m, axis=0, keepdims=True)

    def body(h, carry):
        for j in range(NJ):
            mcur = m_s[j]
            m = None
            acc = None
            for c in range(NC):
                acc = pv_chunk(h, j, c, mcur, acc)
                m = qk_chunk(h + 1, j, c, m)
            pv_finish(h, j, acc)
            m_s[j] = jnp.max(m, axis=0, keepdims=True)
        return carry

    jax.lax.fori_loop(0, H - 1, body, 0)

    xrow = jax.lax.broadcasted_iota(jnp.int32, (DA, TR), 0)
    xaug = jnp.where(xrow == 0, 1.0, 0.0).astype(bf16)

    def pv_last(j):
        mcur = m_s[j]
        acc = None
        for c in range(NC):
            acc = pv_chunk(H - 1, j, c, mcur, acc)
        pv_finish(H - 1, j, acc)

    def pre(r):
        cols = pl.ds(r * TR, TR)
        ot = _up(ot_s[:, :, cols].reshape(H * HP // 2, TR))
        attn = jnp.dot(_up(wot_s[...]), ot, preferred_element_type=f32)
        h1 = xt_ref[:, cols].astype(f32) + attn
        xn2 = jnp.concatenate([_layernorm_t(h1).astype(bf16), xaug], axis=0)
        return h1, xn2

    NF = 14
    FB = F // NF
    pv_last(0)
    nxt = pre(0)
    for r in range(NR):
        cols = pl.ds(r * TR, TR)
        h1, xn2 = nxt
        hids = []
        mcur = m_s[r + 1] if r + 1 < NR else None
        acc = None
        for t in range(NF):
            hid = jnp.dot(_up(w1t_s[t * FB // 2:(t + 1) * FB // 2, :]), xn2,
                          preferred_element_type=f32)
            hid = jnp.maximum(hid, 0.0)
            hids.append((hid * hid).astype(bf16))
            if r + 1 < NR:
                for c in range(t * NC // NF, (t + 1) * NC // NF):
                    acc = pv_chunk(H - 1, r + 1, c, mcur, acc)
        if r + 1 < NR:
            pv_finish(H - 1, r + 1, acc)
            nxt = pre(r + 1)
        hid = jnp.concatenate(hids, axis=0)
        y = jnp.dot(_up(w2t_s[...]), hid, preferred_element_type=f32)
        b2c = jnp.concatenate([b2c_s[...]] * (TR // 128), axis=1)
        out_ref[:, cols] = (h1 + y + b2c).astype(out_ref.dtype)
        out_copy(r).start()
    for r in range(NR):
        out_copy(r).wait()


@jax.jit
def pallas_sequential_preLN__softmax_full_mha__dense_activation_squared_relu__prompt_kernel(
    A_x: jax.Array,
    A_wqkv: jax.Array,
    A_wo: jax.Array,
    B_x: jax.Array,
    B_w1: jax.Array,
    B_b1: jax.Array,
    B_w2: jax.Array,
    B_b2: jax.Array,
):
    del B_x
    B, S, D = A_x.shape
    F = B_w1.shape[1]
    assert B == 1 and TR == TQ
    out_t = pl.pallas_call(
        _kernel,
        out_shape=jax.ShapeDtypeStruct((D, S), A_x.dtype),
        in_specs=[pl.BlockSpec(memory_space=pl.ANY)] * 7,
        out_specs=pl.BlockSpec(memory_space=pl.ANY),
        scratch_shapes=[
            pltpu.VMEM((D, S), bf16),
            pltpu.VMEM((D, 3 * D), bf16),
            pltpu.VMEM((D, D), bf16),
            pltpu.VMEM((D, F), bf16),
            pltpu.VMEM((F // 128, 128), bf16),
            pltpu.VMEM((D, F), bf16),
            pltpu.VMEM((1, D), bf16),
            pltpu.VMEM((D, S), bf16),
            pltpu.SemaphoreType.DMA((8 + S // TR,)),
            pltpu.VMEM((3 * D // 2, D), u32),
            pltpu.VMEM((D // 2, H * HP), u32),
            pltpu.VMEM((F // 2, D + DA), u32),
            pltpu.VMEM((D // 2, F), u32),
            pltpu.VMEM((D, 128), f32),
            pltpu.VMEM((H // HG, S // 2, 128), u32),
            pltpu.VMEM((H, 64, S), u32),
            pltpu.VMEM((H, HP // 2, S), u32),
            pltpu.VMEM((H, HP // 2, S), u32),
            pltpu.VMEM((S // TQ, S, TQ), f32),
            pltpu.VMEM((S // TQ, 1, TQ), f32),
        ],
        compiler_params=pltpu.CompilerParams(vmem_limit_bytes=100 * 2**20),
    )(A_x.reshape(S, D).T, A_wqkv, A_wo, B_w1, B_b1.reshape(F // 128, 128), B_w2.T,
      B_b2.reshape(1, D))
    return out_t.T.reshape(B, S, D)
```

```python
import math

import jax
import jax.numpy as jnp
import jax.experimental.pallas as pl
import jax.experimental.pallas.tpu as pltpu

H = 16
HP = 32
HG = 4
HB = 2
EPS = 1e-5
TR = 512
TQ = 512
CK = 128
DA = 16
WA = 384
DEFER = 1
NQ = 8
PVS = 13
F2SPLIT = [0, 112, 224, 336, 448]
F2LAST = [0, 224, 384, 448]
PR = 64
FILL = 3
K1 = 1
K2 = 2
K20 = 8
WB = 768
ZH = 11
K10 = [8, 4, 4, 4]
GSPLIT = [0, 2, 3, 4, 5, 6, 7, 8, 9, 10, 11, 12]
G_WC = 4
G_WB = 2
G_X1 = 11

f32, bf16, u32 = jnp.float32, jnp.bfloat16, jnp.uint32


def _pk(x):
    return pltpu.bitcast(x, u32)


def _up(x):
    return pltpu.bitcast(x, bf16)


def _colmean(x, k):
    parts = [x[i:i + 8] for i in range(0, x.shape[0], 8)]
    accs = parts[:k]
    for i in range(k, len(parts)):
        accs[i % k] = accs[i % k] + parts[i]
    while len(accs) > 1:
        accs = [accs[i] + accs[i + 1] if i + 1 < len(accs) else accs[i]
                for i in range(0, len(accs), 2)]
    return jnp.sum(accs[0], axis=0, keepdims=True) * (1.0 / x.shape[0])


def _layernorm_t(x, k):
    m = _colmean(x, k)
    d = m - x
    v = _colmean(d * d, k)
    return (x - m) * jax.lax.rsqrt(v + EPS)


def _kernel(xt_hbm, wqkv_hbm, wo_hbm, w1_hbm, b1_hbm, w2t_hbm, b2_hbm, out_hbm,
            xt_ref, wqkv_ref, wo_ref, w1_ref, w2t_ref, out_ref,
            wt_s, wot_s, w1t_s, w2t_s, b2c_s, k_s, qt_s, vt_s, ot_s, s_s, z_s, m_s,
            b1_ref, b2_ref, sems):
    D, S = xt_ref.shape
    F = w1_ref.shape[1]
    DH = D // H
    PAD = HP - DH
    GW = HG * DH
    NG = H // HG
    NJ = S // TQ
    NC = S // CK
    NR = S // TR
    NF = F // 128
    qscale = (DH ** -0.5) * math.log2(math.e)

    def win(h):
        return h * DH - (PAD if h % 2 else 0)

    def qwin(i):
        return (i * DH) // 16 * 16, -(-((i + 1) * DH) // 16) * 16

    copies = dict(
        wa=(wqkv_hbm.at[:, 0:WA], wqkv_ref.at[:, 0:WA]),
        x0=(xt_hbm.at[:, 0:TR], xt_ref.at[:, 0:TR]),
        wb=(wqkv_hbm.at[:, WA:WB], wqkv_ref.at[:, WA:WB]),
        wc=(wqkv_hbm.at[:, WB:3 * D], wqkv_ref.at[:, WB:3 * D]),
        x1=(xt_hbm.at[:, TR:S], xt_ref.at[:, TR:S]),
        b1=(b1_hbm, b1_ref), b2=(b2_hbm, b2_ref), wo=(wo_hbm, wo_ref),
        w1=(w1_hbm, w1_ref), w2=(w2t_hbm, w2t_ref))
    copies = {n: pltpu.make_async_copy(s, d, sems.at[min(i, 5)])
              for i, (n, (s, d)) in enumerate(copies.items())}
    out_copies = []

    def out_copy(rows, cols):
        cp = pltpu.make_async_copy(out_ref.at[rows, cols], out_hbm.at[rows, cols], sems.at[0])
        out_copies.append(cp)
        return cp

    def ln1(r):
        return _layernorm_t(xt_ref[:, pl.ds(r * TR, TR)].astype(f32), K1).astype(bf16)

    for cp in copies.values():
        cp.start()
    for h in range(H):
        if h == ZH:
            copies["wa"].wait()
            wt_s[0:WA // 2, :] = _pk(wqkv_ref[:, 0:WA].T)
        lo, hi = qwin(h % HG)
        if lo > 0:
            qt_s[h, 0:lo // 2, :] = jnp.zeros((lo // 2, S), u32)
        qt_s[h, hi // 2:64, :] = jnp.zeros((64 - hi // 2, S), u32)
    z_s[...] = jnp.zeros_like(z_s)
    copies["x0"].wait()

    xn0 = jnp.concatenate(
        [_layernorm_t(xt_ref[:, t * 128:(t + 1) * 128].astype(f32), K10[t]).astype(bf16)
         for t in range(TR // 128)], axis=1)
    hrow = jax.lax.broadcasted_iota(jnp.int32, (HP, TR), 0)
    fill_even = jnp.where(hrow == DH, 1.0, 0.0)
    fill_odd = jnp.where(hrow == 0, 1.0, 0.0)
    zg = jnp.zeros((128 - GW, TR), bf16)

    def prep_small():
        wo = wo_ref[...].astype(f32)
        wrow = jax.lax.broadcasted_iota(jnp.int32, (HP, D), 0)
        wo_p = jnp.concatenate(
            [jnp.where((wrow < DH) if h % 2 == 0 else (wrow >= PAD),
                       wo[win(h):win(h) + HP], 0.0) for h in range(H)], axis=0)
        wot_s[...] = _pk(wo_p.T.astype(bf16))
        b2c_s[...] = jnp.broadcast_to(b2_ref[...].astype(f32), (128, D)).T

    def proj_store(r, gi, y):
        cols = pl.ds(r * TR, TR)
        kind, g = divmod(gi, NG)
        if kind == 0:
            qg = y * qscale
            for i in range(HG):
                lo, hi = qwin(i)
                grow = jax.lax.broadcasted_iota(jnp.int32, (hi - lo, TR), 0)
                msk = (grow >= i * DH - lo) & (grow < (i + 1) * DH - lo)
                qm = jnp.where(msk, qg[lo:hi], 0.0).astype(bf16)
                qt_s[g * HG + i, lo // 2:hi // 2, cols] = _pk(qm)
        elif kind == 1:
            k_s[g, pl.ds(r * TR // 2, TR // 2), :] = _pk(
                jnp.concatenate([y.astype(bf16), zg], axis=0).T)
        else:
            for i in range(HG):
                vw = y[win(i):win(i) + HP]
                if i % 2 == 0:
                    vw = jnp.where(hrow < DH, vw, fill_even)
                else:
                    vw = jnp.where(hrow >= PAD, vw, fill_odd)
                vt_s[g * HG + i, :, cols] = _pk(vw.astype(bf16))

    def proj(r, g0, g1, xn):
        y = jnp.dot(_up(wt_s[g0 * GW // 2:g1 * GW // 2, :]), xn, preferred_element_type=f32)
        for gi in range(g0, g1):
            proj_store(r, gi, y[(gi - g0) * GW:(gi - g0 + 1) * GW])

    for g0, g1 in zip(GSPLIT[:-1], GSPLIT[1:]):
        if g0 == G_WB:
            copies["wb"].wait()
            wt_s[WA // 2:WB // 2, :] = _pk(wqkv_ref[:, WA:WB].T)
        if g0 == G_WC:
            copies["wc"].wait()
            wt_s[WB // 2:3 * D // 2, :] = _pk(wqkv_ref[:, WB:3 * D].T)
        if g0 == G_X1:
            copies["x1"].wait()
        proj(0, g0, g1, xn0)
    for r in range(1, NR):
        proj(r, 0, 3 * NG, ln1(r))

    def qk_chunk(h, u, c, m):
        j = u % NJ
        qt = _up(qt_s[h, :, pl.ds(j * TQ, TQ)])
        k = _up(k_s[h // HG, pl.ds(c * CK // 2, CK // 2), :])
        s = jnp.dot(k, qt, preferred_element_type=f32)
        s_s[u, pl.ds(c * CK, CK), :] = s
        mc = jnp.max(s.reshape(CK // 8, 8, TQ), axis=0)
        return mc if m is None else jnp.maximum(m, mc)

    def pv_chunk(h, u, c, m, acc):
        s = s_s[u, pl.ds(c * CK, CK), :]
        p = jnp.exp2(s - m).astype(bf16)
        vt = _up(vt_s[h, :, pl.ds(c * CK, CK)])
        o = jnp.dot(vt, p, preferred_element_type=f32)
        return o if acc is None else acc + o

    def pv_finish(h, u, acc):
        if HB % 2 == 0:
            l = acc[DH:DH + 1, :] if (u // NJ) % 2 == 0 else acc[0:1, :]
        else:
            l = jnp.where(h % 2 == 0, acc[DH:DH + 1, :], acc[0:1, :])
        ot_s[h, :, pl.ds((u % NJ) * TQ, TQ)] = _pk((acc / l).astype(bf16))

    def prep_steps():
        b1 = b1_ref[...].astype(f32)
        arow = jax.lax.broadcasted_iota(jnp.int32, (DA, 128), 0)
        for t in range(NF):
            aug = jnp.where(arow == 0, b1[t:t + 1, :], 0.0).astype(bf16)
            w1a = jnp.concatenate([w1_ref[:, t * 128:(t + 1) * 128], aug], axis=0)
            w1t_s[t * 64:(t + 1) * 64, :] = _pk(w1a.T)
            yield
        prep_small()

    prep = prep_steps()
    for u in range(HB * NJ):
        if u == 1:
            for n in ("b1", "b2", "wo", "w1", "w2"):
                copies[n].wait()
        m = None
        for c in range(NC):
            m = qk_chunk(u // NJ, u, c, m)
            if u >= 1 and c % 2 == 1:
                next(prep, None)
        m_s[u] = jnp.max(m, axis=0, keepdims=True)

    NIT = H // HB - 1

    W2R = D // NIT

    def body(it, carry):
        r0 = pl.multiple_of(it * W2R, W2R)
        w2t_s[pl.ds(pl.multiple_of(it * (W2R // 2), W2R // 2), W2R // 2), :] = _pk(
            w2t_ref[pl.ds(r0, W2R), :])
        pending = None
        for u in range(HB * NJ):
            h = it * HB + u // NJ
            mcur = m_s[u]
            m = None
            acc = z_s[...] if u > 0 else None
            for c in range(NC):
                acc = pv_chunk(h, u, c, mcur, acc)
                m = qk_chunk(h + HB, u, c, m)
                if c == DEFER and pending is not None:
                    pv_finish(*pending)
            pending = (h, u, acc)
            m_s[u] = jnp.max(m, axis=0, keepdims=True)
        pv_finish(*pending)
        return carry

    jax.lax.fori_loop(0, NIT, body, 0)

    xrow = jax.lax.broadcasted_iota(jnp.int32, (DA, 128), 0)
    xaug = jnp.where(xrow == 0, 1.0, 0.0).astype(bf16)
    HE = H - HG
    NT = TR // 128

    def pv_steps(r):
        pending = None
        for b in range(HB):
            u = b * NJ + r
            h = H - HB + b
            mcur = m_s[u]
            acc = z_s[...]
            for c in range(NC):
                acc = pv_chunk(h, u, c, mcur, acc)
                if c == DEFER and pending is not None:
                    pv_finish(*pending)
                if b == HB - 1 and c == NC - 1:
                    pv_finish(h, u, acc)
                yield
            pending = (h, u, acc)

    def advance(gen, n):
        for _ in range(n):
            next(gen, None)

    def oproj(r, rows, h0, h1):
        cols = pl.ds(r * TR, TR)
        ot = _up(ot_s[h0:h1, :, cols].reshape((h1 - h0) * HP // 2, TR))
        w = _up(wot_s[rows[0] // 2:rows[1] // 2, h0 * HP:h1 * HP])
        return jnp.dot(w, ot, preferred_element_type=f32)

    def part(r, rows, h1=HE):
        return (xt_ref[rows[0]:rows[1], pl.ds(r * TR, TR)].astype(f32)
                + oproj(r, rows, 0, h1))

    def norm2(h1, t, k=K2):
        ht = h1[:, t * 128:(t + 1) * 128]
        return jnp.concatenate([_layernorm_t(ht, k).astype(bf16), xaug], axis=0)

    def part_steps(r, out):
        for a in range(0, D, PR):
            rows = (a, min(a + PR, D))
            acc = xt_ref[rows[0]:rows[1], pl.ds(r * TR, TR)].astype(f32)
            for g in range(HE // HG):
                acc = acc + oproj(r, rows, g * HG, (g + 1) * HG)
                if g == HE // HG - 1:
                    out.append(acc)
                yield True

    gen = pv_steps(0)
    parts0, parts1 = [], []
    g0, g1 = part_steps(0, parts0), part_steps(1, parts1)
    for q in range(HB * NC):
        if next(g0, None) is None:
            next(g1, None)
        advance(gen, 1)
    advance(g1, FILL)
    h1 = jnp.concatenate(parts0, axis=0) + oproj(0, (0, D), HE, H)
    xn2 = norm2(h1, 0, K20)
    for _ in g1:
        pass
    pnext = jnp.concatenate(parts1, axis=0)
    FQ = F // NQ
    for r in range(NR):
        gen = pv_steps(r + 1) if r + 1 < NR else iter(())
        h1cur = h1
        hids = []
        for t in range(NT):
            pieces = []
            for q in range(NQ):
                hid = jnp.dot(_up(w1t_s[q * FQ // 2:(q + 1) * FQ // 2, :]), xn2,
                              preferred_element_type=f32)
                hid = jnp.maximum(hid, 0.0)
                pieces.append((hid * hid).astype(bf16))
                advance(gen, 1)
                if q == NQ // 2 - 1 and t + 1 < NT:
                    xn2n = norm2(h1cur, t + 1)
            hids.append(jnp.concatenate(pieces, axis=0))
            if t + 1 == NT and r + 1 < NR:
                advance(gen, HB * NC)
                if pnext is None:
                    h1 = part(r + 1, (0, D), H)
                else:
                    h1 = pnext + oproj(r + 1, (0, D), HE, H)
                pnext = None
                xn2n = norm2(h1, 0)
            xn2 = xn2n
            if t % 2 == 1:
                hid = jnp.concatenate(hids[t - 1:t + 1], axis=1)
                c0 = (t - 1) * 128
                cols = pl.ds(r * TR + c0, 256)
                last = r + 1 == NR and t + 1 == NT
                splits = F2LAST if last else F2SPLIT
                for a, b in zip(splits[:-1], splits[1:]):
                    y = jnp.dot(_up(w2t_s[a // 2:b // 2, :]), hid, preferred_element_type=f32)
                    b2c = jnp.concatenate([b2c_s[a:b]] * 2, axis=1)
                    out_ref[a:b, cols] = (h1cur[a:b, c0:c0 + 256] + y + b2c).astype(out_ref.dtype)
                    advance(gen, 1)
                    if last:
                        out_copy(pl.ds(a, b - a), cols).start()
                if not last:
                    out_copy(pl.ds(0, D), cols).start()
    for cp in out_copies:
        cp.wait()


@jax.jit
def pallas_sequential_preLN__softmax_full_mha__dense_activation_squared_relu__prompt_kernel(
    A_x: jax.Array,
    A_wqkv: jax.Array,
    A_wo: jax.Array,
    B_x: jax.Array,
    B_w1: jax.Array,
    B_b1: jax.Array,
    B_w2: jax.Array,
    B_b2: jax.Array,
):
    del B_x
    B, S, D = A_x.shape
    F = B_w1.shape[1]
    assert B == 1 and TR == TQ
    out_t = pl.pallas_call(
        _kernel,
        out_shape=jax.ShapeDtypeStruct((D, S), A_x.dtype),
        in_specs=[pl.BlockSpec(memory_space=pl.ANY)] * 7,
        out_specs=pl.BlockSpec(memory_space=pl.ANY),
        scratch_shapes=[
            pltpu.VMEM((D, S), bf16),
            pltpu.VMEM((D, 3 * D), bf16),
            pltpu.VMEM((D, D), bf16),
            pltpu.VMEM((D, F), bf16),
            pltpu.VMEM((D, F), bf16),
            pltpu.VMEM((D, S), bf16),
            pltpu.VMEM((3 * D // 2, D), u32),
            pltpu.VMEM((D // 2, H * HP), u32),
            pltpu.VMEM((F // 2, D + DA), u32),
            pltpu.VMEM((D // 2, F), u32),
            pltpu.VMEM((D, 128), f32),
            pltpu.VMEM((H // HG, S // 2, 128), u32),
            pltpu.VMEM((H, 64, S), u32),
            pltpu.VMEM((H, HP // 2, S), u32),
            pltpu.VMEM((H, HP // 2, S), u32),
            pltpu.VMEM((HB * S // TQ, S, TQ), f32),
            pltpu.VMEM((HP, TQ), f32),
            pltpu.VMEM((HB * S // TQ, 1, TQ), f32),
            pltpu.VMEM((F // 128, 128), bf16),
            pltpu.VMEM((1, D), bf16),
            pltpu.SemaphoreType.DMA((6,)),
        ],
        compiler_params=pltpu.CompilerParams(vmem_limit_bytes=100 * 2**20),
    )(A_x.reshape(S, D).T, A_wqkv, A_wo, B_w1, B_b1.reshape(F // 128, 128), B_w2.T,
      B_b2.reshape(1, D))
    return out_t.T.reshape(B, S, D)
```

```python
import math

import jax
import jax.numpy as jnp
import jax.experimental.pallas as pl
import jax.experimental.pallas.tpu as pltpu

H = 16
HP = 32
HG = 4
HB = 2
EPS = 1e-5
TR = 512
TQ = 512
CK = 128
DA = 16
WA = 384
DEFER = 1
FQ = 128
F2SPLIT = [0, 112, 224]
F2LAST = [0, 80, 160, 224]
OPD = 36
LNT = [38, 40, 42, 44]
FORM0 = 47
FORMN = 2
FILL2 = [1, 1, 1]
FILL3 = 5
FORMN0 = 2
W1R = 8
W2S = 16
PM = 4
PC = 3
NMS = 2
PR = 64
FILL = 3
K1 = 1
K11 = 1
XN1 = 3
P_X2 = 2
XN = 2
XGAP = 2
G_WS = 4
WSROWS = [0]
K2 = 1
K20 = 2
WB = 896
ZH = 11
K10 = [4, 2, 2, 2]
GORDER = [0, 2, 4, 5, 6, 3, 7, 8, 9, 10, 11]
G_WC = 7
G_WB = 2
G_X1 = 7

BIASED = (2, 3, 5, 6)

f32, bf16, u32 = jnp.float32, jnp.bfloat16, jnp.uint32


def _pk(x):
    return pltpu.bitcast(x, u32)


def _zip(lo, hi):
    return pltpu.pack_elementwise([lo, hi], packed_dtype=bf16)


def _zip16(x):
    lo, hi = [jnp.concatenate([x[g:g + 8] for g in range(e, x.shape[0], 16)], axis=0)
              for e in (0, 8)]
    return _zip(lo, hi)


def _unzip(p):
    return jnp.concatenate(
        [pltpu.unpack_elementwise(p, index=i, packed_dtype=bf16, unpacked_dtype=f32)
         for i in range(2)], axis=0)


def _up(x):
    return pltpu.bitcast(x, bf16)


def _colmean(parts, k):
    accs = parts[:k]
    for i in range(k, len(parts)):
        accs[i % k] = accs[i % k] + parts[i]
    while len(accs) > 1:
        accs = [accs[i] + accs[i + 1] if i + 1 < len(accs) else accs[i]
                for i in range(0, len(accs), 2)]
    return jnp.sum(accs[0], axis=0, keepdims=True) * (1.0 / (8 * len(parts)))


def _stats_t(x, k, zero=None):
    c = jnp.broadcast_to(x[0:1], (8, x.shape[1]))
    if zero is not None:
        c = c + zero
    d = [x[i:i + 8] - c for i in range(0, x.shape[0], 8)]
    m = _colmean(d, k)
    v = _colmean([e * e for e in d], k) - m * m
    return c[0:1] + m, jax.lax.rsqrt(v + EPS)


def _layernorm_t(x, k):
    m, rs = _stats_t(x, k)
    return (x - m) * rs


def _lhs_ops(a11, a12, a21, a22):
    return [a11 + a22, a21 + a22, a11, a22, a11 + a12, a21 - a11, a12 - a22]


def _rhs_ops(b11, b12, b21, b22):
    return [b11 + b22, b11, b12 - b22, b21 - b11, b22, b11 + b12, b21 + b22]


def _kernel(xt_hbm, wqkv_hbm, wo_hbm, w1_hbm, b1_hbm, w2t_hbm, b2_hbm, out_hbm,
            xt_ref, wqkv_ref, wo_ref, w1_ref, w2t_ref, out_ref,
            wt_s, aq_s, wot_s, w1t_s, a1_s, b2c_s, k_s, qt_s, vt_s, ot_s, s_s, z_s, m_s, ms_s, u_s, ul_s, t_s, a2_s,
            b1_ref, b2_ref, o_s, sems):
    D, S = xt_ref.shape
    F = w1_ref.shape[1]
    DH = D // H
    PAD = HP - DH
    GW = HG * DH
    NG = H // HG
    NJ = S // TQ
    NC = S // CK
    NR = S // TR
    NF = F // 128
    qscale = (DH ** -0.5) * math.log2(math.e)

    def win(h):
        return h * DH - (PAD if h % 2 else 0)

    def qwin(i):
        return (i * DH) // 16 * 16, -(-((i + 1) * DH) // 16) * 16

    copies = dict(
        wa=(wqkv_hbm.at[:, 0:WA], wqkv_ref.at[:, 0:WA]),
        x0=(xt_hbm.at[:, 0:TR], xt_ref.at[:, 0:TR]),
        wb=(wqkv_hbm.at[:, WA:WB], wqkv_ref.at[:, WA:WB]),
        wc=(wqkv_hbm.at[:, WB:3 * D], wqkv_ref.at[:, WB:3 * D]),
        x1=(xt_hbm.at[:, TR:2 * TR], xt_ref.at[:, TR:2 * TR]),
        x2=(xt_hbm.at[:, 2 * TR:S], xt_ref.at[:, 2 * TR:S]),
        b1=(b1_hbm, b1_ref), b2=(b2_hbm, b2_ref), wo=(wo_hbm, wo_ref),
        w1=(w1_hbm, w1_ref), w2=(w2t_hbm, w2t_ref.at[0:D]))
    sem_of = dict(wa=0, x0=1, wb=2, wc=3, x1=3, x2=4)
    copies = {n: pltpu.make_async_copy(s, d, sems.at[sem_of.get(n, 5)])
              for n, (s, d) in copies.items()}
    out_copies = []

    def out_copy(rows, cols):
        cp = pltpu.make_async_copy(out_ref.at[rows, cols], out_hbm.at[rows, cols], sems.at[0])
        out_copies.append(cp)
        return cp

    def after(v):
        bits = pltpu.bitcast(v[0:8, 0:128], u32) & pltpu.bitcast(z_s[0:8, 0:128], u32)
        return pltpu.bitcast(bits, f32)

    def wt_prep(a, b):
        wt_s[a // 2:b // 2, :] = _pk(_up(_zip16(wqkv_ref[:, a:b].astype(f32))).T)

    for cp in copies.values():
        cp.start()
    for h in range(H):
        if h == ZH:
            copies["wa"].wait()
            wt_prep(0, WA)
        lo, hi = qwin(h % HG)
        if lo > 0:
            qt_s[h, 0:lo // 2, :] = jnp.zeros((lo // 2, S), u32)
        qt_s[h, hi // 2:64, :] = jnp.zeros((64 - hi // 2, S), u32)
    z_s[...] = jnp.zeros_like(z_s)
    o_s[0] = 0
    copies["x0"].wait()

    o = o_s[0]
    xn0 = _up(jnp.concatenate(
        [_zip16(_layernorm_t(xt_ref[:, t * 128:(t + 1) * 128].astype(f32), K10[t]))
         for t in range(TR // 128)], axis=1))
    def prep_small():
        wo = wo_ref[...].astype(f32)
        wrow = jax.lax.broadcasted_iota(jnp.int32, (HP, D), 0)
        wo_p = jnp.concatenate(
            [jnp.where((wrow < DH) if h % 2 == 0 else (wrow >= PAD),
                       wo[win(h):win(h) + HP], 0.0) for h in range(H)], axis=0)
        wot_s[...] = _pk(wo_p.T.astype(bf16))
        b2c_s[...] = jnp.broadcast_to(b2_ref[...].astype(f32), (128, D)).T

    def proj_store(c0, gi, y):
        n = y.shape[1]
        cols = pl.ds(c0, n)
        kind, g = divmod(gi, NG)
        if kind == 0:
            qg = y * qscale
            for i in range(HG):
                lo, hi = qwin(i)
                grow = jax.lax.broadcasted_iota(jnp.int32, (hi - lo, n), 0)
                msk = (grow >= i * DH - lo) & (grow < (i + 1) * DH - lo)
                qm = jnp.where(msk, qg[lo:hi], 0.0).astype(bf16)
                qt_s[g * HG + i, lo // 2:hi // 2, cols] = _pk(qm)
        elif kind == 1:
            k_s[g, pl.ds(c0 // 2, n // 2), :] = _pk(
                jnp.concatenate([y, jnp.zeros((128 - GW, n), f32)], axis=0).astype(bf16).T)
        else:
            hrow = jax.lax.broadcasted_iota(jnp.int32, (HP, n), 0)
            for i in range(HG):
                vw = y[win(i):win(i) + HP]
                if i % 2 == 0:
                    vw = jnp.where(hrow < DH, vw, jnp.where(hrow == DH, 1.0, 0.0))
                else:
                    vw = jnp.where(hrow >= PAD, vw, jnp.where(hrow == 0, 1.0, 0.0))
                vt_s[g * HG + i, :, cols] = _pk(vw.astype(bf16))

    HT = TR // 2
    NT = TR // 128
    KA, KB = 256, D - 256
    SHORT = (3, 4, 6)
    GH = GW // 2

    def pair_rows(p):
        g = (p // 2) * NG + p % 2
        return g, g + NG // 2

    def wsum_steps():
        for p in range(3 * NG // 2):
            for a in range(0, GH, 8):
                v = yield
                wt_s[3 * D // 2:3 * D // 2 + 8, 0:128] = pltpu.bitcast(v[0:8, 0:128], u32)
                blks = []
                for g in pair_rows(p):
                    w = wt_s[pl.ds(pl.multiple_of(o + (g * GH + a), 8), 8), :]
                    blks += [_unzip(w[:, :KA]), _unzip(jnp.concatenate(
                        [w[:, KA:], jnp.zeros((8, KA - KB), u32)], axis=1))]
                for i, op in enumerate(_lhs_ops(*blks)):
                    if i not in (2, 3):
                        aq_s[i - 2 * (i > 3), p * GH + a:p * GH + a + 8, :] = _zip(op[:8], op[8:])
        while True:
            yield

    def xtile(r, rows, t):
        return xt_ref[rows[0]:rows[1], r * TR + t * 128:r * TR + (t + 1) * 128].astype(f32)

    def xform_steps(r, k, n):
        st = []
        for t in range(NT):
            z = after((yield))
            st.append(_stats_t(xtile(r, (0, D), t), k, z))
        for _ in range(XGAP):
            yield
        q = 0
        for t in range(NT // 2):
            for a in range(0, KA, 16):
                if q % n == 0:
                    z = after((yield))
                q += 1
                blks = []
                for i in range(2):
                    for tt in (t, t + NT // 2):
                        if i * KA + a < D:
                            mu = st[tt][0] + z
                            x = xtile(r, (i * KA + a, i * KA + a + 16), tt)
                            blks.append((x - jnp.concatenate([mu, mu], axis=0)) * st[tt][1])
                if a < KB:
                    ops = _rhs_ops(*blks)
                else:
                    ops = [blks[0], blks[0], blks[1], None, None, blks[0] + blks[1], None]
                for i, op in enumerate(ops):
                    if op is not None:
                        t_s[r % 2][0, i, a // 2:a // 2 + 8, t * 128:(t + 1) * 128] = _zip(op[:8], op[8:])
        while True:
            yield

    def started(gen):
        next(gen)
        return gen

    wsum = started(wsum_steps())
    xform = started(xform_steps(1, K11, XN1))
    for n, g0 in enumerate(GORDER):
        g1 = g0 + (2 if n == 0 else 1)
        n = n + 1 if n else 0
        if n == G_WB:
            copies["wb"].wait()
            wt_prep(WA, WB)
        if n == G_WC:
            copies["wc"].wait()
            copies["x1"].wait()
            wt_prep(WB, 3 * D)
        y = jnp.dot(_up(wt_s[g0 * GH:g1 * GH, :]), xn0, preferred_element_type=f32)
        for gi in range(g0, g1):
            proj_store(0, gi, y[(gi - g0) * GW:(gi - g0 + 1) * GW])
        for t in range(NT):
            if n >= G_WS:
                for a in WSROWS:
                    wsum.send(y[a:a + 8, t * 128:(t + 1) * 128])
            if n >= G_X1:
                xform.send(y[56:64, t * 128:(t + 1) * 128])
    for r in range(1, NR):
        xform = started(xform_steps(r + 1, K1, XN)) if r + 1 < NR else None

        def tick(v):
            wsum.send(v)
            if xform is not None and (r > 1 or p >= P_X2):
                xform.send(v)

        for p in range(3 * NG // 2):
            if r == 1 and p == P_X2:
                copies["x2"].wait()
            ms = [m.at[:, 0:GW] for m in ms_s[p % NMS * 9:][:5]]
            gs = pair_rows(p)

            def mm(i):
                kk = KB if i in SHORT else KA
                if i == 2:
                    w = wt_s[gs[0] * GH:(gs[0] + 1) * GH, 0:KA]
                elif i == 3:
                    w = wt_s[gs[1] * GH:(gs[1] + 1) * GH, KA:D]
                else:
                    w = aq_s[i - 2 * (i > 3), p * GH:(p + 1) * GH, 0:kk]
                return jnp.dot(_up(w), _up(t_s[r % 2][o, i, 0:kk // 2, :]),
                               preferred_element_type=f32)

            m = mm(0); ms[0][0] = m; tick(m)
            m = mm(2); ms[2][0] = m; tick(m)
            m = mm(1); ms[1][0] = m; tick(m)
            m = mm(4); ms[4][0] = m; proj_store(r * TR + HT, gs[0], m + ms[2][o]); tick(m)
            m = mm(3); ms[3][0] = m; proj_store(r * TR, gs[1], m + ms[1][o]); tick(m)
            m = mm(5)
            proj_store(r * TR + HT, gs[1], ((m + ms[0][o]) + ms[2][o]) - ms[1][o]); tick(m)
            m = mm(6)
            proj_store(r * TR, gs[0], ((m + ms[0][o]) + ms[3][o]) - ms[4][o]); tick(m)

    def qk_chunk(h, u, c, m):
        j = u % NJ
        qt = _up(qt_s[h, :, pl.ds(j * TQ, TQ)])
        k = _up(k_s[h // HG, pl.ds(c * CK // 2, CK // 2), :])
        s = jnp.dot(k, qt, preferred_element_type=f32)
        s_s[u, pl.ds(c * CK, CK), :] = s
        mc = jnp.max(s.reshape(CK // 8, 8, TQ), axis=0)
        return mc if m is None else jnp.maximum(m, mc)

    def pv_chunk(h, u, c, m, acc):
        s = s_s[u, pl.ds(c * CK, CK), :]
        p = jnp.exp2(s - m).astype(bf16)
        vt = _up(vt_s[h, :, pl.ds(c * CK, CK)])
        o = jnp.dot(vt, p, preferred_element_type=f32)
        return o if acc is None else acc + o

    def pv_finish(h, u, acc):
        if HB % 2 == 0:
            l = acc[DH:DH + 1, :] if (u // NJ) % 2 == 0 else acc[0:1, :]
        else:
            l = jnp.where(h % 2 == 0, acc[DH:DH + 1, :], acc[0:1, :])
        ot_s[h, :, pl.ds((u % NJ) * TQ, TQ)] = _pk((acc / l).astype(bf16))

    D2, F2 = D // 2, F // 2

    D4 = D // 4

    def prep_steps():
        b1 = b1_ref[...].astype(f32)
        arow = jax.lax.broadcasted_iota(jnp.int32, (DA, 128), 0)
        for t in range(NF):
            for j in range(2):
                aug = jnp.where(arow == 2 * (t // (NF // 2)) + j, b1[t:t + 1, :], 0.0).astype(bf16)
                w = w1_ref[j * D2:(j + 1) * D2, t * 128:(t + 1) * 128].astype(f32)
                w = jnp.concatenate([_up(_zip(w[:D4], w[D4:])), aug], axis=0)
                w1t_s[j, t * 64:(t + 1) * 64, :] = _pk(_unzip(_pk(w.T)).astype(bf16))
                yield
        prep_small()
        xrow = jax.lax.broadcasted_iota(jnp.int32, (DA, TR // 2), 0)
        xaug = _pk(jnp.where(xrow < 4, 1.0, 0.0).astype(bf16))
        for t in t_s:
            for i in BIASED:
                t[0, i, D4:D4 + DA // 2, :] = xaug

    prep = prep_steps()
    for u in range(HB * NJ):
        if u == 1:
            for n in ("b1", "b2", "wo", "w1", "w2"):
                copies[n].wait()
        m = None
        for c in range(NC):
            m = qk_chunk(u // NJ, u, c, m)
            if u >= 1 and c % 2 == 1:
                next(prep, None)
        m_s[u] = jnp.max(m, axis=0, keepdims=True)

    NIT = H // HB - 1

    W2R = D2 // NIT

    def loop_prep(it):
        for q in range(0, 64, W1R):
            v = yield
            w1t_s[0, F2:F2 + 8, 0:128] = pltpu.bitcast(v[0:8, 0:128], u32)
            blks = [_unzip(w1t_s[j, pl.ds(pl.multiple_of(i * (F2 // 2) + it * 64 + q, W1R), W1R), :])
                    for i in range(2) for j in range(2)]
            for i, op in enumerate(_lhs_ops(*blks)):
                if i not in (2, 3):
                    a1_s[i - 2 * (i > 3), pl.ds(pl.multiple_of(it * 64 + q, W1R), W1R), :] = _zip(
                        op[:W1R], op[W1R:])
        for q in range(NF // 2):
            for a in range(0, W2R, W2S):
                v = yield
                w2t_ref[D:D + 16, 0:128] = pltpu.bitcast(v[0:8, 0:128], bf16)
                blks = [_unzip(_pk(w2t_ref[pl.ds(pl.multiple_of(i * D2 + it * W2R + a, W2S), W2S),
                                           j * F2 + q * 128:j * F2 + (q + 1) * 128]))
                        for i in range(2) for j in range(2)]
                for i, op in enumerate(_lhs_ops(*blks)):
                    a2_s[i, pl.ds(pl.multiple_of((it * W2R + a) // 2, W2S // 2), W2S // 2),
                         q * 128:(q + 1) * 128] = _zip(op[:W2S // 2], op[W2S // 2:])
        while True:
            yield

    def body(it, carry):
        prep = loop_prep(it)
        next(prep)
        pending = None
        for u in range(HB * NJ):
            h = it * HB + u // NJ
            mcur = m_s[u]
            m = None
            acc = z_s[...] if u > 0 else None
            for c in range(NC):
                acc = pv_chunk(h, u, c, mcur, acc)
                m = qk_chunk(h + HB, u, c, m)
                if c == DEFER and pending is not None:
                    pv_finish(*pending)
                if c % PM == PC:
                    prep.send(m)
            pending = (h, u, acc)
            m_s[u] = jnp.max(m, axis=0, keepdims=True)
        pv_finish(*pending)
        return carry

    jax.lax.fori_loop(0, NIT, body, 0)

    o = o_s[0]
    HE = H - HG

    def pv_steps(r):
        pending = None
        for b in range(HB):
            u = b * NJ + r
            h = H - HB + b
            mcur = m_s[u]
            acc = z_s[...]
            for c in range(NC):
                acc = pv_chunk(h, u, c, mcur, acc)
                if c == DEFER and pending is not None:
                    pv_finish(*pending)
                if b == HB - 1 and c == NC - 1:
                    pv_finish(h, u, acc)
                yield
            pending = (h, u, acc)

    def advance(gen, n):
        v = None
        for _ in range(n):
            v = next(gen, None)
        return v

    def oproj(r, rows, h0, h1):
        cols = pl.ds(r * TR, TR)
        ot = _up(ot_s[h0:h1, :, cols].reshape((h1 - h0) * HP // 2, TR))
        w = _up(wot_s[rows[0] // 2:rows[1] // 2, h0 * HP:h1 * HP])
        return jnp.dot(w, ot, preferred_element_type=f32)

    def part(r, rows, h1=HE):
        return (xt_ref[rows[0]:rows[1], pl.ds(r * TR, TR)].astype(f32)
                + oproj(r, rows, 0, h1))

    def stats2(h1, t, k, dep):
        return _stats_t(h1[:, t * 128:(t + 1) * 128], k, None if dep is None else after(dep))

    def form_steps(r, h1, st, n):
        z = None
        for t in range(NT // 2):
            for q, a in enumerate(range(0, D4, 8)):
                if (t * (D4 // 8) + q) % n == 0:
                    z = after((yield))
                blks = []
                for i in range(2):
                    for tt in (t, t + NT // 2):
                        x = jnp.concatenate(
                            [h1[i * D2 + e * D4 + a:i * D2 + e * D4 + a + 8, tt * 128:(tt + 1) * 128]
                             for e in range(2)], axis=0)
                        mu = st[tt][0] + z
                        blks.append((x - jnp.concatenate([mu, mu], axis=0)) * st[tt][1])
                for i, op in enumerate(_rhs_ops(*blks)):
                    t_s[r % 2][0, i, a:a + 8, t * 128:(t + 1) * 128] = _zip(op[:8], op[8:])
        while True:
            yield

    def part_steps(r, out):
        for a in range(0, D, PR):
            rows = (a, min(a + PR, D))
            acc = xt_ref[rows[0]:rows[1], pl.ds(r * TR, TR)].astype(f32)
            for g in range(HE // HG):
                acc = acc + oproj(r, rows, g * HG, (g + 1) * HG)
                if g == HE // HG - 1:
                    out.append(acc)
                yield acc

    def strassen(mm, tick, fin):
        m3 = mm(2); tick(m3)
        m5 = mm(4)
        fin(0, 1, m5 + m3); tick(m5)
        m2 = mm(1); tick(m2)
        m4 = mm(3)
        fin(1, 0, m4 + m2); tick(m4)
        m1 = mm(0); tick(m1)
        m7 = mm(6)
        fin(0, 0, ((m7 + m1) + m4) - m5); tick(m7)
        m6 = mm(5)
        fin(1, 1, ((m6 + m1) + m3) - m2); tick(m6)

    gen = pv_steps(0)
    parts = [[] for _ in range(3)]
    fill = (x for r in range(3) for x in part_steps(r, parts[r]))
    for q in range(HB * NC):
        advance(fill, 1)
        advance(gen, 1)
    advance(fill, FILL)
    h1 = jnp.concatenate(parts[0], axis=0) + oproj(0, (0, D), HE, H)
    st = [stats2(h1, 0, K20, None)]
    for t in range(1, NT):
        st.append(stats2(h1, t, K20, advance(fill, FILL2[t - 1])))
    advance(fill, FILL3)
    form = form_steps(0, h1, st, FORMN0)
    next(form)
    for v in fill:
        form.send(v)
    for r in range(NR):
        gen = pv_steps(r + 1) if r + 1 < NR else iter(())
        h1cur = h1
        st = []
        state = dict(n=0)

        def tick(v):
            state["n"] += 1
            n = state["n"]
            advance(gen, 1)
            if r + 1 < NR:
                if n == OPD:
                    if r + 1 < len(parts):
                        state["h1"] = (jnp.concatenate(parts[r + 1], axis=0)
                                       + oproj(r + 1, (0, D), HE, H))
                    else:
                        state["h1"] = part(r + 1, (0, D), H)
                if n in LNT:
                    st.append(stats2(state["h1"], len(st), K2, v))
                if n == FORM0:
                    state["form"] = form_steps(r + 1, state["h1"], st, FORMN)
                    next(state["form"])
                if n >= FORM0:
                    state["form"].send(v)

        def act(c):
            c = jnp.maximum(c, 0.0)
            return c * c

        late = [lambda: None] * 2
        for a in range(0, F2, FQ):
            ms = ms_s[(a // FQ) % NMS * 9:][:9]
            rows = slice(a // 2, (a + FQ) // 2)

            def mm(i):
                kk = D2 + DA if i in BIASED else D2
                if i in (2, 3):
                    w = w1t_s[i - 2, pl.ds((i - 2) * F2 // 2 + a // 2, FQ // 2), 0:kk]
                else:
                    w = a1_s[i - 2 * (i > 3), rows, 0:kk]
                return jnp.dot(_up(w), _up(t_s[r % 2][o, i, 0:kk // 2, :]),
                               preferred_element_type=f32)

            def put(i, v, p=a // FQ):
                v = _zip(v[:FQ // 2], v[FQ // 2:])
                if (p + 1) * FQ < F2:
                    u_s[0, i, p * FQ // 2:(p + 1) * FQ // 2, :] = v
                else:
                    ul_s[i][0] = v

            m = mm(0); ms[0][0] = m; late.pop(0)(); tick(m)
            m = mm(2); ms[2][0] = m; late.pop(0)(); tick(m)
            m = mm(1); ms[1][0] = m; tick(m)
            m = mm(4); ms[4][0] = m; ms[6][0] = act(m + ms[2][o]); tick(m)
            m = mm(3); ms[3][0] = m; ms[7][0] = act(m + ms[1][o]); tick(m)
            m = mm(5)
            b = act(((m + ms[0][o]) + ms[2][o]) - ms[1][o])
            ms[8][0] = b
            put(4, b); put(2, ms[6][o] - b); tick(m)
            m = mm(6)
            b = act(((m + ms[0][o]) + ms[3][o]) - ms[4][o])
            ms[5][0] = b
            put(1, b); put(3, ms[7][o] - b); put(5, b + ms[6][o]); tick(m)
            late = [lambda ms=ms, put=put: put(6, ms[7][o] + ms[8][o]),
                    lambda ms=ms, put=put: put(0, ms[5][o] + ms[8][o])]
        for f in late:
            f()
        split = F2LAST if r + 1 == NR else F2SPLIT
        for a, b in zip(split[:-1], split[1:]):
            last = r + 1 == NR and b == D2

            def fin2(i, j, c):
                rows = slice(i * D2 + a, i * D2 + b)
                cols = pl.ds(r * TR + j * HT, HT)
                b2c = jnp.concatenate([b2c_s[rows]] * (HT // 128), axis=1)
                out_ref[rows, cols] = (h1cur[rows, j * HT:(j + 1) * HT] + c + b2c).astype(out_ref.dtype)
                if r + 1 == NR and i == j:
                    out_copy(pl.ds(i * D2 + a, b - a), pl.ds(r * TR, TR)).start()

            strassen(lambda i: jnp.dot(_up(a2_s[i, a // 2:b // 2, :]), _up(jnp.concatenate([u_s[o, i], ul_s[i][o]], axis=0)),
                                       preferred_element_type=f32), tick, fin2)
        if r + 1 < NR:
            out_copy(pl.ds(0, D), pl.ds(r * TR, TR)).start()
            h1 = state["h1"]
    for cp in out_copies:
        cp.wait()


@jax.jit
def pallas_sequential_preLN__softmax_full_mha__dense_activation_squared_relu__prompt_kernel(
    A_x: jax.Array,
    A_wqkv: jax.Array,
    A_wo: jax.Array,
    B_x: jax.Array,
    B_w1: jax.Array,
    B_b1: jax.Array,
    B_w2: jax.Array,
    B_b2: jax.Array,
):
    del B_x
    B, S, D = A_x.shape
    F = B_w1.shape[1]
    assert B == 1 and TR == TQ
    out_t = pl.pallas_call(
        _kernel,
        out_shape=jax.ShapeDtypeStruct((D, S), A_x.dtype),
        in_specs=[pl.BlockSpec(memory_space=pl.ANY)] * 7,
        out_specs=pl.BlockSpec(memory_space=pl.ANY),
        scratch_shapes=[
            pltpu.VMEM((D, S), bf16),
            pltpu.VMEM((D, 3 * D), bf16),
            pltpu.VMEM((D, D), bf16),
            pltpu.VMEM((D, F), bf16),
            pltpu.VMEM((D + 32, F), bf16),
            pltpu.VMEM((D, S), bf16),
            pltpu.VMEM((3 * D // 2 + 8, D), u32),
            pltpu.VMEM((5, 3 * D // 4, 256), u32),
            pltpu.VMEM((D // 2, H * HP), u32),
            pltpu.VMEM((2, F // 2 + 16, D // 2 + DA), u32),
            pltpu.VMEM((5, F // 4, D // 2 + DA), u32),
            pltpu.VMEM((D, 128), f32),
            pltpu.VMEM((H // HG, S // 2, 128), u32),
            pltpu.VMEM((H, 64, S), u32),
            pltpu.VMEM((H, HP // 2, S), u32),
            pltpu.VMEM((H, HP // 2, S), u32),
            pltpu.VMEM((HB * S // TQ, S, TQ), f32),
            pltpu.VMEM((HP, TQ), f32),
            pltpu.VMEM((HB * S // TQ, 1, TQ), f32),
            [pltpu.VMEM((1, FQ, TR // 2), f32)] * (9 * NMS),
            pltpu.VMEM((1, 7, F // 4 - FQ // 2, TR // 2), u32),
            [pltpu.VMEM((1, FQ // 2, TR // 2), u32)] * 7,
            [pltpu.VMEM((1, 7, 128, TR // 2), u32)] * 2,
            pltpu.VMEM((7, D // 4, F // 2), u32),
            pltpu.VMEM((F // 128, 128), bf16),
            pltpu.VMEM((1, D), bf16),
            pltpu.SMEM((1,), jnp.int32),
            pltpu.SemaphoreType.DMA((6,)),
        ],
        compiler_params=pltpu.CompilerParams(vmem_limit_bytes=100 * 2**20),
    )(A_x.reshape(S, D).T, A_wqkv, A_wo, B_w1, B_b1.reshape(F // 128, 128), B_w2.T,
      B_b2.reshape(1, D))
    return out_t.T.reshape(B, S, D)
```

```python
import math

import jax
import jax.numpy as jnp
import jax.experimental.pallas as pl
import jax.experimental.pallas.tpu as pltpu

H = 16
HP = 32
HG = 4
HB = 2
EPS = 1e-5
TR = 512
TQ = 512
CK = 128
DA = 16
WA = 384
DEFER = 1
FQ = 128
F2SPLIT = [0, 112, 224]
F2LAST = [0, 80, 160, 224]
OPD = 36
LNT = [38, 40, 42, 44]
FORM0 = 47
FORMN = 2
FILL2 = [1, 1, 1]
FILL3 = 5
FORMN0 = 2
W2S = 32
WG = 8
NMS = 2
PR = 64
FILL = 3
K1 = 1
K11 = 1
XN1 = 3
P_X2 = 2
XN = 2
XGAP = 2
G_WS = 4
WSROWS = [0]
K2 = 1
K20 = 2
WB = 896
ZH = 11
K10 = [4, 2, 2, 2]
GORDER = [0, 2, 4, 5, 6, 3, 7, 8, 9, 10, 11]
G_WC = 7
G_WB = 2
G_X1 = 7

BIASED = (2, 3, 5, 6)

f32, bf16, u32 = jnp.float32, jnp.bfloat16, jnp.uint32


def _pk(x):
    return pltpu.bitcast(x, u32)


def _zip(lo, hi):
    return pltpu.pack_elementwise([lo, hi], packed_dtype=bf16)


def _zip16(x):
    lo, hi = [jnp.concatenate([x[g:g + 8] for g in range(e, x.shape[0], 16)], axis=0)
              for e in (0, 8)]
    return _zip(lo, hi)


def _unzip(p):
    return jnp.concatenate(
        [pltpu.unpack_elementwise(p, index=i, packed_dtype=bf16, unpacked_dtype=f32)
         for i in range(2)], axis=0)


def _up(x):
    return pltpu.bitcast(x, bf16)


def _colmean(parts, k):
    accs = parts[:k]
    for i in range(k, len(parts)):
        accs[i % k] = accs[i % k] + parts[i]
    while len(accs) > 1:
        accs = [accs[i] + accs[i + 1] if i + 1 < len(accs) else accs[i]
                for i in range(0, len(accs), 2)]
    return jnp.sum(accs[0], axis=0, keepdims=True) * (1.0 / (8 * len(parts)))


def _stats_t(x, k, zero=None):
    c = jnp.broadcast_to(x[0:1], (8, x.shape[1]))
    if zero is not None:
        c = c + zero
    d = [x[i:i + 8] - c for i in range(0, x.shape[0], 8)]
    m = _colmean(d, k)
    v = _colmean([e * e for e in d], k) - m * m
    return c[0:1] + m, jax.lax.rsqrt(v + EPS)


def _layernorm_t(x, k):
    m, rs = _stats_t(x, k)
    return (x - m) * rs


def _lhs_ops(a11, a12, a21, a22):
    return [a11 + a22, a21 + a22, a11, a22, a11 + a12, a21 - a11, a12 - a22]


def _rhs_ops(b11, b12, b21, b22):
    return [b11 + b22, b11, b12 - b22, b21 - b11, b22, b11 + b12, b21 + b22]


def _kernel(xt_hbm, wqkv_hbm, wo_hbm, w1_hbm, b1_hbm, w2t_hbm, b2_hbm, out_hbm,
            xt_ref, wqkv_ref, wo_ref, w1_ref, w2t_ref, out_ref,
            wt_s, aq_s, wot_s, w1t_s, a1_s, b2c_s, k_s, qt_s, vt_s, ot_s, s_s, z_s, m_s, ms_s, u_s, ul_s, t_s, a2_s,
            b1_ref, b2_ref, o_s, sems):
    D, S = xt_ref.shape
    F = w1_ref.shape[1]
    DH = D // H
    PAD = HP - DH
    GW = HG * DH
    NG = H // HG
    NJ = S // TQ
    NC = S // CK
    NR = S // TR
    NF = F // 128
    qscale = (DH ** -0.5) * math.log2(math.e)

    def win(h):
        return h * DH - (PAD if h % 2 else 0)

    def qwin(i):
        return (i * DH) // 16 * 16, -(-((i + 1) * DH) // 16) * 16

    copies = dict(
        wa=(wqkv_hbm.at[:, 0:WA], wqkv_ref.at[:, 0:WA]),
        x0=(xt_hbm.at[:, 0:TR], xt_ref.at[:, 0:TR]),
        wb=(wqkv_hbm.at[:, WA:WB], wqkv_ref.at[:, WA:WB]),
        wc=(wqkv_hbm.at[:, WB:3 * D], wqkv_ref.at[:, WB:3 * D]),
        x1=(xt_hbm.at[:, TR:2 * TR], xt_ref.at[:, TR:2 * TR]),
        x2=(xt_hbm.at[:, 2 * TR:S], xt_ref.at[:, 2 * TR:S]),
        b1=(b1_hbm, b1_ref), b2=(b2_hbm, b2_ref), wo=(wo_hbm, wo_ref),
        w1=(w1_hbm, w1_ref.at[0:D]), w2=(w2t_hbm, w2t_ref.at[0:D]))
    sem_of = dict(wa=0, x0=1, wb=2, wc=3, x1=3, x2=4)
    copies = {n: pltpu.make_async_copy(s, d, sems.at[sem_of.get(n, 5)])
              for n, (s, d) in copies.items()}
    out_copies = []

    def out_copy(rows, cols):
        cp = pltpu.make_async_copy(out_ref.at[rows, cols], out_hbm.at[rows, cols], sems.at[0])
        out_copies.append(cp)
        return cp

    def after(v):
        bits = pltpu.bitcast(v[0:8, 0:128], u32) & pltpu.bitcast(z_s[0:8, 0:128], u32)
        return pltpu.bitcast(bits, f32)

    def wt_prep(a, b):
        wt_s[a // 2:b // 2, :] = _pk(_up(_zip16(wqkv_ref[:, a:b].astype(f32))).T)

    for cp in copies.values():
        cp.start()
    for h in range(H):
        if h == ZH:
            copies["wa"].wait()
            wt_prep(0, WA)
        lo, hi = qwin(h % HG)
        if lo > 0:
            qt_s[h, 0:lo // 2, :] = jnp.zeros((lo // 2, S), u32)
        qt_s[h, hi // 2:64, :] = jnp.zeros((64 - hi // 2, S), u32)
    z_s[...] = jnp.zeros_like(z_s)
    o_s[0] = 0
    copies["x0"].wait()

    o = o_s[0]
    xn0 = _up(jnp.concatenate(
        [_zip16(_layernorm_t(xt_ref[:, t * 128:(t + 1) * 128].astype(f32), K10[t]))
         for t in range(TR // 128)], axis=1))
    def prep_small():
        wo = wo_ref[...].astype(f32)
        wrow = jax.lax.broadcasted_iota(jnp.int32, (HP, D), 0)
        wo_p = jnp.concatenate(
            [jnp.where((wrow < DH) if h % 2 == 0 else (wrow >= PAD),
                       wo[win(h):win(h) + HP], 0.0) for h in range(H)], axis=0)
        wot_s[...] = _pk(wo_p.T.astype(bf16))
        b2c_s[...] = jnp.broadcast_to(b2_ref[...].astype(f32), (128, D)).T

    def proj_store(c0, gi, y):
        n = y.shape[1]
        cols = pl.ds(c0, n)
        kind, g = divmod(gi, NG)
        if kind == 0:
            qg = y * qscale
            for i in range(HG):
                lo, hi = qwin(i)
                grow = jax.lax.broadcasted_iota(jnp.int32, (hi - lo, n), 0)
                msk = (grow >= i * DH - lo) & (grow < (i + 1) * DH - lo)
                qm = jnp.where(msk, qg[lo:hi], 0.0).astype(bf16)
                qt_s[g * HG + i, lo // 2:hi // 2, cols] = _pk(qm)
        elif kind == 1:
            k_s[g, pl.ds(c0 // 2, n // 2), :] = _pk(
                jnp.concatenate([y, jnp.zeros((128 - GW, n), f32)], axis=0).astype(bf16).T)
        else:
            hrow = jax.lax.broadcasted_iota(jnp.int32, (HP, n), 0)
            for i in range(HG):
                vw = y[win(i):win(i) + HP]
                if i % 2 == 0:
                    vw = jnp.where(hrow < DH, vw, jnp.where(hrow == DH, 1.0, 0.0))
                else:
                    vw = jnp.where(hrow >= PAD, vw, jnp.where(hrow == 0, 1.0, 0.0))
                vt_s[g * HG + i, :, cols] = _pk(vw.astype(bf16))

    HT = TR // 2
    NT = TR // 128
    KA, KB = 256, D - 256
    SHORT = (3, 4, 6)
    GH = GW // 2

    def pair_rows(p):
        g = (p // 2) * NG + p % 2
        return g, g + NG // 2

    def wsum_steps():
        for p in range(3 * NG // 2):
            for a in range(0, GH, 8):
                v = yield
                wt_s[3 * D // 2:3 * D // 2 + 8, 0:128] = pltpu.bitcast(v[0:8, 0:128], u32)
                blks = []
                for g in pair_rows(p):
                    w = wt_s[pl.ds(pl.multiple_of(o + (g * GH + a), 8), 8), :]
                    blks += [_unzip(w[:, :KA]), _unzip(jnp.concatenate(
                        [w[:, KA:], jnp.zeros((8, KA - KB), u32)], axis=1))]
                for i, op in enumerate(_lhs_ops(*blks)):
                    if i not in (2, 3):
                        aq_s[i - 2 * (i > 3), p * GH + a:p * GH + a + 8, :] = _zip(op[:8], op[8:])
        while True:
            yield

    def xtile(r, rows, t):
        return xt_ref[rows[0]:rows[1], r * TR + t * 128:r * TR + (t + 1) * 128].astype(f32)

    def xform_steps(r, k, n):
        st = []
        for t in range(NT):
            z = after((yield))
            st.append(_stats_t(xtile(r, (0, D), t), k, z))
        for _ in range(XGAP):
            yield
        q = 0
        for t in range(NT // 2):
            for a in range(0, KA, 16):
                if q % n == 0:
                    z = after((yield))
                q += 1
                blks = []
                for i in range(2):
                    for tt in (t, t + NT // 2):
                        if i * KA + a < D:
                            mu = st[tt][0] + z
                            x = xtile(r, (i * KA + a, i * KA + a + 16), tt)
                            blks.append((x - jnp.concatenate([mu, mu], axis=0)) * st[tt][1])
                if a < KB:
                    ops = _rhs_ops(*blks)
                else:
                    ops = [blks[0], blks[0], blks[1], None, None, blks[0] + blks[1], None]
                for i, op in enumerate(ops):
                    if op is not None:
                        t_s[r % 2][0, i, a // 2:a // 2 + 8, t * 128:(t + 1) * 128] = _zip(op[:8], op[8:])
        while True:
            yield

    def started(gen):
        next(gen)
        return gen

    wsum = started(wsum_steps())
    xform = started(xform_steps(1, K11, XN1))
    for n, g0 in enumerate(GORDER):
        g1 = g0 + (2 if n == 0 else 1)
        n = n + 1 if n else 0
        if n == G_WB:
            copies["wb"].wait()
            wt_prep(WA, WB)
        if n == G_WC:
            copies["wc"].wait()
            copies["x1"].wait()
            wt_prep(WB, 3 * D)
        y = jnp.dot(_up(wt_s[g0 * GH:g1 * GH, :]), xn0, preferred_element_type=f32)
        for gi in range(g0, g1):
            proj_store(0, gi, y[(gi - g0) * GW:(gi - g0 + 1) * GW])
        for t in range(NT):
            if n >= G_WS:
                for a in WSROWS:
                    wsum.send(y[a:a + 8, t * 128:(t + 1) * 128])
            if n >= G_X1:
                xform.send(y[56:64, t * 128:(t + 1) * 128])
    for r in range(1, NR):
        xform = started(xform_steps(r + 1, K1, XN)) if r + 1 < NR else None

        def tick(v):
            wsum.send(v)
            if xform is not None and (r > 1 or p >= P_X2):
                xform.send(v)

        for p in range(3 * NG // 2):
            if r == 1 and p == P_X2:
                copies["x2"].wait()
            ms = [m.at[:, 0:GW] for m in ms_s[p % NMS * 9:][:5]]
            gs = pair_rows(p)

            def mm(i):
                kk = KB if i in SHORT else KA
                if i == 2:
                    w = wt_s[gs[0] * GH:(gs[0] + 1) * GH, 0:KA]
                elif i == 3:
                    w = wt_s[gs[1] * GH:(gs[1] + 1) * GH, KA:D]
                else:
                    w = aq_s[i - 2 * (i > 3), p * GH:(p + 1) * GH, 0:kk]
                return jnp.dot(_up(w), _up(t_s[r % 2][o, i, 0:kk // 2, :]),
                               preferred_element_type=f32)

            m = mm(0); ms[0][0] = m; tick(m)
            m = mm(2); ms[2][0] = m; tick(m)
            m = mm(1); ms[1][0] = m; tick(m)
            m = mm(4); ms[4][0] = m; proj_store(r * TR + HT, gs[0], m + ms[2][o]); tick(m)
            m = mm(3); ms[3][0] = m; proj_store(r * TR, gs[1], m + ms[1][o]); tick(m)
            m = mm(5)
            proj_store(r * TR + HT, gs[1], ((m + ms[0][o]) + ms[2][o]) - ms[1][o]); tick(m)
            m = mm(6)
            proj_store(r * TR, gs[0], ((m + ms[0][o]) + ms[3][o]) - ms[4][o]); tick(m)

    def qk_chunk(h, u, c, m, gate=None):
        j = u % NJ
        qt = _up(qt_s[h, :, pl.ds(j * TQ, TQ)])
        k = k_s[h // HG, pl.ds(c * CK // 2, CK // 2), :]
        if gate is not None:
            k = jnp.concatenate([k[0:8] | pltpu.bitcast(after(gate), u32), k[8:]], axis=0)
        k = _up(k)
        s = jnp.dot(k, qt, preferred_element_type=f32)
        s_s[u, pl.ds(c * CK, CK), :] = s
        mc = jnp.max(s.reshape(CK // 8, 8, TQ), axis=0)
        return mc if m is None else jnp.maximum(m, mc)

    def pv_chunk(h, u, c, m, acc):
        s = s_s[u, pl.ds(c * CK, CK), :]
        p = jnp.exp2(s - m).astype(bf16)
        vt = _up(vt_s[h, :, pl.ds(c * CK, CK)])
        o = jnp.dot(vt, p, preferred_element_type=f32)
        return o if acc is None else acc + o

    def pv_finish(h, u, acc):
        if HB % 2 == 0:
            l = acc[DH:DH + 1, :] if (u // NJ) % 2 == 0 else acc[0:1, :]
        else:
            l = jnp.where(h % 2 == 0, acc[DH:DH + 1, :], acc[0:1, :])
        ot_s[h, :, pl.ds((u % NJ) * TQ, TQ)] = _pk((acc / l).astype(bf16))

    D2, F2 = D // 2, F // 2

    D4 = D // 4

    def w1_block(t, i, j, v):
        b1 = b1_ref[...].astype(f32)
        arow = jax.lax.broadcasted_iota(jnp.int32, (DA, 128), 0)
        tt = i * (NF // 2) + t
        aug = jnp.where(arow == 2 * i + j, b1[tt:tt + 1, :], 0.0).astype(bf16)
        w1_ref[D:D + 16, 0:128] = pltpu.bitcast(v[0:8, 0:128], bf16)
        w = w1_ref[pl.ds(pl.multiple_of(o + j * D2, 16), D2), tt * 128:(tt + 1) * 128].astype(f32)
        w = jnp.concatenate([_up(_zip(w[:D4], w[D4:])), aug], axis=0)
        w1t_s[j, tt * 64:(tt + 1) * 64, :] = _pk(_unzip(_pk(w.T)).astype(bf16))

    def w1_sums(a, v):
        w1t_s[0, F2:F2 + 8, 0:128] = pltpu.bitcast(v[0:8, 0:128], u32)
        blks = [_unzip(w1t_s[j, pl.ds(pl.multiple_of(o + (i * (F2 // 2) + a), 8), 8), :])
                for i in range(2) for j in range(2)]
        for i, op in enumerate(_lhs_ops(*blks)):
            if i not in (2, 3):
                a1_s[i - 2 * (i > 3), a:a + 8, :] = _zip(op[:8], op[8:])

    def w2_steps():
        for q in range(NF // 2):
            for a in range(0, D2, W2S):
                v = yield
                w2t_ref[D:D + 16, 0:128] = pltpu.bitcast(v[0:8, 0:128], bf16)
                blks = [_unzip(_pk(w2t_ref[pl.ds(pl.multiple_of(o + (i * D2 + a), W2S), W2S),
                                           j * F2 + q * 128:j * F2 + (q + 1) * 128]))
                        for i in range(2) for j in range(2)]
                for i, op in enumerate(_lhs_ops(*blks)):
                    a2_s[i, a // 2:(a + W2S) // 2, q * 128:(q + 1) * 128] = _zip(
                        op[:W2S // 2], op[W2S // 2:])
        while True:
            yield

    w2sum = started(w2_steps())
    for u in range(HB * NJ):
        if u == 1:
            for n in ("b1", "b2", "wo", "w1", "w2"):
                copies[n].wait()
            prep_small()
            xrow = jax.lax.broadcasted_iota(jnp.int32, (DA, TR // 2), 0)
            xaug = _pk(jnp.where(xrow < 4, 1.0, 0.0).astype(bf16))
            for t in t_s:
                for i in BIASED:
                    t[0, i, D4:D4 + DA // 2, :] = xaug
        m = None
        for c in range(NC):
            gate = None
            if u >= 1 and c == WG:
                gate = w1t_s[0, pl.ds(pl.multiple_of(o + (u - 1) * 64, 8), 8), 0:128]
            m = qk_chunk(u // NJ, u, c, m, gate)
            if u >= 1:
                if c < 4:
                    w1_block(u - 1, c // 2, c % 2, m)
                if c < WG:
                    w2sum.send(m)
                elif c < WG + 8:
                    w1_sums((u - 1) * 64 + (c - WG) * 8, m)
        m_s[u] = jnp.max(m, axis=0, keepdims=True)

    NIT = H // HB - 1

    def body(it, carry):
        pending = None
        for u in range(HB * NJ):
            h = it * HB + u // NJ
            mcur = m_s[u]
            m = None
            acc = z_s[...] if u > 0 else None
            for c in range(NC):
                acc = pv_chunk(h, u, c, mcur, acc)
                m = qk_chunk(h + HB, u, c, m)
                if c == DEFER and pending is not None:
                    pv_finish(*pending)
            pending = (h, u, acc)
            m_s[u] = jnp.max(m, axis=0, keepdims=True)
        pv_finish(*pending)
        return carry

    jax.lax.fori_loop(0, NIT, body, 0)

    o = o_s[0]
    HE = H - HG

    def pv_steps(r):
        pending = None
        for b in range(HB):
            u = b * NJ + r
            h = H - HB + b
            mcur = m_s[u]
            acc = z_s[...]
            for c in range(NC):
                acc = pv_chunk(h, u, c, mcur, acc)
                if c == DEFER and pending is not None:
                    pv_finish(*pending)
                if b == HB - 1 and c == NC - 1:
                    pv_finish(h, u, acc)
                yield
            pending = (h, u, acc)

    def advance(gen, n):
        v = None
        for _ in range(n):
            v = next(gen, None)
        return v

    def oproj(r, rows, h0, h1):
        cols = pl.ds(r * TR, TR)
        ot = _up(ot_s[h0:h1, :, cols].reshape((h1 - h0) * HP // 2, TR))
        w = _up(wot_s[rows[0] // 2:rows[1] // 2, h0 * HP:h1 * HP])
        return jnp.dot(w, ot, preferred_element_type=f32)

    def part(r, rows, h1=HE):
        return (xt_ref[rows[0]:rows[1], pl.ds(r * TR, TR)].astype(f32)
                + oproj(r, rows, 0, h1))

    def stats2(h1, t, k, dep):
        return _stats_t(h1[:, t * 128:(t + 1) * 128], k, None if dep is None else after(dep))

    def form_steps(r, h1, st, n):
        z = None
        for t in range(NT // 2):
            for q, a in enumerate(range(0, D4, 8)):
                if (t * (D4 // 8) + q) % n == 0:
                    z = after((yield))
                blks = []
                for i in range(2):
                    for tt in (t, t + NT // 2):
                        x = jnp.concatenate(
                            [h1[i * D2 + e * D4 + a:i * D2 + e * D4 + a + 8, tt * 128:(tt + 1) * 128]
                             for e in range(2)], axis=0)
                        mu = st[tt][0] + z
                        blks.append((x - jnp.concatenate([mu, mu], axis=0)) * st[tt][1])
                for i, op in enumerate(_rhs_ops(*blks)):
                    t_s[r % 2][0, i, a:a + 8, t * 128:(t + 1) * 128] = _zip(op[:8], op[8:])
        while True:
            yield

    def part_steps(r, out):
        for a in range(0, D, PR):
            rows = (a, min(a + PR, D))
            acc = xt_ref[rows[0]:rows[1], pl.ds(r * TR, TR)].astype(f32)
            for g in range(HE // HG):
                acc = acc + oproj(r, rows, g * HG, (g + 1) * HG)
                if g == HE // HG - 1:
                    out.append(acc)
                yield acc

    def strassen(mm, tick, fin):
        m3 = mm(2); tick(m3)
        m5 = mm(4)
        fin(0, 1, m5 + m3); tick(m5)
        m2 = mm(1); tick(m2)
        m4 = mm(3)
        fin(1, 0, m4 + m2); tick(m4)
        m1 = mm(0); tick(m1)
        m7 = mm(6)
        fin(0, 0, ((m7 + m1) + m4) - m5); tick(m7)
        m6 = mm(5)
        fin(1, 1, ((m6 + m1) + m3) - m2); tick(m6)

    gen = pv_steps(0)
    parts = [[] for _ in range(3)]
    fill = (x for r in range(3) for x in part_steps(r, parts[r]))
    for q in range(HB * NC):
        advance(fill, 1)
        advance(gen, 1)
    advance(fill, FILL)
    h1 = jnp.concatenate(parts[0], axis=0) + oproj(0, (0, D), HE, H)
    st = [stats2(h1, 0, K20, None)]
    for t in range(1, NT):
        st.append(stats2(h1, t, K20, advance(fill, FILL2[t - 1])))
    advance(fill, FILL3)
    form = form_steps(0, h1, st, FORMN0)
    next(form)
    for v in fill:
        form.send(v)
    for r in range(NR):
        gen = pv_steps(r + 1) if r + 1 < NR else iter(())
        h1cur = h1
        st = []
        state = dict(n=0)

        def tick(v):
            state["n"] += 1
            n = state["n"]
            advance(gen, 1)
            if r + 1 < NR:
                if n == OPD:
                    if r + 1 < len(parts):
                        state["h1"] = (jnp.concatenate(parts[r + 1], axis=0)
                                       + oproj(r + 1, (0, D), HE, H))
                    else:
                        state["h1"] = part(r + 1, (0, D), H)
                if n in LNT:
                    st.append(stats2(state["h1"], len(st), K2, v))
                if n == FORM0:
                    state["form"] = form_steps(r + 1, state["h1"], st, FORMN)
                    next(state["form"])
                if n >= FORM0:
                    state["form"].send(v)

        def act(c):
            c = jnp.maximum(c, 0.0)
            return c * c

        late = [lambda: None] * 2
        for a in range(0, F2, FQ):
            ms = ms_s[(a // FQ) % NMS * 9:][:9]
            rows = slice(a // 2, (a + FQ) // 2)

            def mm(i):
                kk = D2 + DA if i in BIASED else D2
                if i in (2, 3):
                    w = w1t_s[i - 2, pl.ds((i - 2) * F2 // 2 + a // 2, FQ // 2), 0:kk]
                else:
                    w = a1_s[i - 2 * (i > 3), rows, 0:kk]
                return jnp.dot(_up(w), _up(t_s[r % 2][o, i, 0:kk // 2, :]),
                               preferred_element_type=f32)

            def put(i, v, p=a // FQ):
                v = _zip(v[:FQ // 2], v[FQ // 2:])
                if (p + 1) * FQ < F2:
                    u_s[0, i, p * FQ // 2:(p + 1) * FQ // 2, :] = v
                else:
                    ul_s[i][0] = v

            m = mm(0); ms[0][0] = m; late.pop(0)(); tick(m)
            m = mm(2); ms[2][0] = m; late.pop(0)(); tick(m)
            m = mm(1); ms[1][0] = m; tick(m)
            m = mm(4); ms[4][0] = m; ms[6][0] = act(m + ms[2][o]); tick(m)
            m = mm(3); ms[3][0] = m; ms[7][0] = act(m + ms[1][o]); tick(m)
            m = mm(5)
            b = act(((m + ms[0][o]) + ms[2][o]) - ms[1][o])
            ms[8][0] = b
            put(4, b); put(2, ms[6][o] - b); tick(m)
            m = mm(6)
            b = act(((m + ms[0][o]) + ms[3][o]) - ms[4][o])
            ms[5][0] = b
            put(1, b); put(3, ms[7][o] - b); put(5, b + ms[6][o]); tick(m)
            late = [lambda ms=ms, put=put: put(6, ms[7][o] + ms[8][o]),
                    lambda ms=ms, put=put: put(0, ms[5][o] + ms[8][o])]
        for f in late:
            f()
        split = F2LAST if r + 1 == NR else F2SPLIT
        for a, b in zip(split[:-1], split[1:]):
            last = r + 1 == NR and b == D2

            def fin2(i, j, c):
                rows = slice(i * D2 + a, i * D2 + b)
                cols = pl.ds(r * TR + j * HT, HT)
                b2c = jnp.concatenate([b2c_s[rows]] * (HT // 128), axis=1)
                out_ref[rows, cols] = (h1cur[rows, j * HT:(j + 1) * HT] + c + b2c).astype(out_ref.dtype)
                if r + 1 == NR and i == j:
                    out_copy(pl.ds(i * D2 + a, b - a), pl.ds(r * TR, TR)).start()

            strassen(lambda i: jnp.dot(_up(a2_s[i, a // 2:b // 2, :]), _up(jnp.concatenate([u_s[o, i], ul_s[i][o]], axis=0)),
                                       preferred_element_type=f32), tick, fin2)
        if r + 1 < NR:
            out_copy(pl.ds(0, D), pl.ds(r * TR, TR)).start()
            h1 = state["h1"]
    for cp in out_copies:
        cp.wait()


@jax.jit
def pallas_sequential_preLN__softmax_full_mha__dense_activation_squared_relu__prompt_kernel(
    A_x: jax.Array,
    A_wqkv: jax.Array,
    A_wo: jax.Array,
    B_x: jax.Array,
    B_w1: jax.Array,
    B_b1: jax.Array,
    B_w2: jax.Array,
    B_b2: jax.Array,
):
    del B_x
    B, S, D = A_x.shape
    F = B_w1.shape[1]
    assert B == 1 and TR == TQ
    out_t = pl.pallas_call(
        _kernel,
        out_shape=jax.ShapeDtypeStruct((D, S), A_x.dtype),
        in_specs=[pl.BlockSpec(memory_space=pl.ANY)] * 7,
        out_specs=pl.BlockSpec(memory_space=pl.ANY),
        scratch_shapes=[
            pltpu.VMEM((D, S), bf16),
            pltpu.VMEM((D, 3 * D), bf16),
            pltpu.VMEM((D, D), bf16),
            pltpu.VMEM((D + 32, F), bf16),
            pltpu.VMEM((D + 32, F), bf16),
            pltpu.VMEM((D, S), bf16),
            pltpu.VMEM((3 * D // 2 + 8, D), u32),
            pltpu.VMEM((5, 3 * D // 4, 256), u32),
            pltpu.VMEM((D // 2, H * HP), u32),
            pltpu.VMEM((2, F // 2 + 16, D // 2 + DA), u32),
            pltpu.VMEM((5, F // 4, D // 2 + DA), u32),
            pltpu.VMEM((D, 128), f32),
            pltpu.VMEM((H // HG, S // 2, 128), u32),
            pltpu.VMEM((H, 64, S), u32),
            pltpu.VMEM((H, HP // 2, S), u32),
            pltpu.VMEM((H, HP // 2, S), u32),
            pltpu.VMEM((HB * S // TQ, S, TQ), f32),
            pltpu.VMEM((HP, TQ), f32),
            pltpu.VMEM((HB * S // TQ, 1, TQ), f32),
            [pltpu.VMEM((1, FQ, TR // 2), f32)] * (9 * NMS),
            pltpu.VMEM((1, 7, F // 4 - FQ // 2, TR // 2), u32),
            [pltpu.VMEM((1, FQ // 2, TR // 2), u32)] * 7,
            [pltpu.VMEM((1, 7, 128, TR // 2), u32)] * 2,
            pltpu.VMEM((7, D // 4, F // 2), u32),
            pltpu.VMEM((F // 128, 128), bf16),
            pltpu.VMEM((1, D), bf16),
            pltpu.SMEM((1,), jnp.int32),
            pltpu.SemaphoreType.DMA((6,)),
        ],
        compiler_params=pltpu.CompilerParams(vmem_limit_bytes=100 * 2**20),
    )(A_x.reshape(S, D).T, A_wqkv, A_wo, B_w1, B_b1.reshape(F // 128, 128), B_w2.T,
      B_b2.reshape(1, D))
    return out_t.T.reshape(B, S, D)
```

```python
import math

import jax
import jax.numpy as jnp
import jax.experimental.pallas as pl
import jax.experimental.pallas.tpu as pltpu

H = 16
HP = 32
HG = 4
HB = 2
EPS = 1e-5
TR = 512
TQ = 512
CK = 128
DA = 16
WA = 384
DEFER = 1
FQ = 128
F2SPLIT = [0, 112, 224]
F2LAST = [0, 80, 160, 224]
OPD = 36
LNT = [38, 40, 42, 44]
FORM0 = 47
FORMN = 2
FILL2 = [1, 1, 1]
FILL3 = 5
FORMN0 = 2
W2S = 16
WG = 8
W2C = range(14)
NPS = (16, 22, 22, 22, 22, 22, 22, 22)
NP = max(NPS)
NCV = 14
RL = 3
GR = 5
GSA = (60, 64)
NPB = (22, 22, 22, 22, 22, 22, 22, 22)
UORD = ((0, 3, 7), (1, 2, 4, 5, 6))
EV = ((72, 127), (129, 238))
GA = 3
CHN = (3, 2)
WD = 3
GS = 124
NMS = 2
PR = 64
FILL = 3
K1 = 1
K11 = 1
XN1 = 3
P_X2 = 2
XN = 2
XGAP = 2
G_WS = 4
WSROWS = [0]
K2 = 1
K20 = 2
WB = 896
ZH = 11
K10 = [4, 2, 2, 2]
GORDER = [0, 2, 4, 5, 6, 3, 7, 8, 9, 10, 11]
G_WC = 7
G_WB = 2
G_X1 = 7

BIASED = (2, 3, 5, 6)

f32, bf16, u32 = jnp.float32, jnp.bfloat16, jnp.uint32


def _pk(x):
    return pltpu.bitcast(x, u32)


def _zip(lo, hi):
    return pltpu.pack_elementwise([lo, hi], packed_dtype=bf16)


def _zip16(x):
    lo, hi = [jnp.concatenate([x[g:g + 8] for g in range(e, x.shape[0], 16)], axis=0)
              for e in (0, 8)]
    return _zip(lo, hi)


def _unzip(p):
    return jnp.concatenate(
        [pltpu.unpack_elementwise(p, index=i, packed_dtype=bf16, unpacked_dtype=f32)
         for i in range(2)], axis=0)


def _up(x):
    return pltpu.bitcast(x, bf16)


def _colmean(parts, k):
    accs = parts[:k]
    for i in range(k, len(parts)):
        accs[i % k] = accs[i % k] + parts[i]
    while len(accs) > 1:
        accs = [accs[i] + accs[i + 1] if i + 1 < len(accs) else accs[i]
                for i in range(0, len(accs), 2)]
    return jnp.sum(accs[0], axis=0, keepdims=True) * (1.0 / (8 * len(parts)))


def _stats_t(x, k, zero=None):
    c = jnp.broadcast_to(x[0:1], (8, x.shape[1]))
    if zero is not None:
        c = c + zero
    d = [x[i:i + 8] - c for i in range(0, x.shape[0], 8)]
    m = _colmean(d, k)
    v = _colmean([e * e for e in d], k) - m * m
    return c[0:1] + m, jax.lax.rsqrt(v + EPS)


def _layernorm_t(x, k):
    m, rs = _stats_t(x, k)
    return (x - m) * rs


def _lhs_ops(a11, a12, a21, a22):
    return [a11 + a22, a21 + a22, a11, a22, a11 + a12, a21 - a11, a12 - a22]


def _rhs_ops(b11, b12, b21, b22):
    return [b11 + b22, b11, b12 - b22, b21 - b11, b22, b11 + b12, b21 + b22]


def _kernel(xt_hbm, wqkv_hbm, wo_hbm, w1_hbm, b1_hbm, w2t_hbm, b2_hbm, out_hbm,
            xt_ref, wqkv_ref, wo_ref, w1_ref, w2t_ref, out_ref,
            wt_s, aq_s, wot_s, w1t_s, a1_s, b2c_s, k_s, qt_s, vt_s, ot_s, s_s, sv_s, qf_s, kf_s, kb_s, z_s, mp_s, m_s, ms_s, u_s, ul_s, t_s, a2_s,
            b1_ref, b2_ref, o_s, sems):
    D, S = xt_ref.shape
    F = w1_ref.shape[1]
    DH = D // H
    PAD = HP - DH
    GW = HG * DH
    NG = H // HG
    NJ = S // TQ
    NC = S // CK
    NR = S // TR
    NF = F // 128
    SMS = [S - 8 * n for n in NPS]
    KV = kf_s.shape[2]
    qscale = (DH ** -0.5) * math.log2(math.e)

    def win(h):
        return h * DH - (PAD if h % 2 else 0)

    def qwin(i):
        return (i * DH) // 16 * 16, -(-((i + 1) * DH) // 16) * 16

    copies = dict(
        wa=(wqkv_hbm.at[:, 0:WA], wqkv_ref.at[:, 0:WA]),
        x0=(xt_hbm.at[:, S - TR:S], xt_ref.at[:, S - TR:S]),
        wb=(wqkv_hbm.at[:, WA:WB], wqkv_ref.at[:, WA:WB]),
        wc=(wqkv_hbm.at[:, WB:3 * D], wqkv_ref.at[:, WB:3 * D]),
        x1=(xt_hbm.at[:, 0:TR], xt_ref.at[:, 0:TR]),
        x2=(xt_hbm.at[:, TR:S - TR], xt_ref.at[:, TR:S - TR]),
        b1=(b1_hbm, b1_ref), b2=(b2_hbm, b2_ref), wo=(wo_hbm, wo_ref),
        w1=(w1_hbm, w1_ref.at[0:D]), w2=(w2t_hbm, w2t_ref.at[0:D]))
    sem_of = dict(wa=0, x0=1, wb=2, wc=3, x1=3, x2=4)
    copies = {n: pltpu.make_async_copy(s, d, sems.at[sem_of.get(n, 5)])
              for n, (s, d) in copies.items()}
    out_copies = []

    def out_copy(rows, cols):
        cp = pltpu.make_async_copy(out_ref.at[rows, cols], out_hbm.at[rows, cols], sems.at[0])
        out_copies.append(cp)
        return cp

    def after(v):
        bits = pltpu.bitcast(v[0:8, 0:128], u32) & pltpu.bitcast(z_s[0:8, 0:128], u32)
        return pltpu.bitcast(bits, f32)

    def wt_prep(a, b):
        wt_s[a // 2:b // 2, :] = _pk(_up(_zip16(wqkv_ref[:, a:b].astype(f32))).T)

    for cp in copies.values():
        cp.start()
    for h in range(H):
        if h == ZH:
            copies["wa"].wait()
            wt_prep(0, WA)
        lo, hi = qwin(h % HG)
        if lo > 0:
            qt_s[h, 0:lo // 2, :] = jnp.zeros((lo // 2, S), u32)
        qt_s[h, hi // 2:64, :] = jnp.zeros((64 - hi // 2, S), u32)
    z_s[...] = jnp.zeros_like(z_s)
    kf_s[H:H + HB] = jnp.zeros((HB,) + kf_s.shape[1:], f32)
    o_s[0] = 0
    copies["x0"].wait()

    o = o_s[0]
    xn0 = _up(jnp.concatenate(
        [_zip16(_layernorm_t(xt_ref[:, S - TR + t * 128:S - TR + (t + 1) * 128].astype(f32), K10[t]))
         for t in range(TR // 128)], axis=1))
    def prep_small():
        wo = wo_ref[...].astype(f32)
        wrow = jax.lax.broadcasted_iota(jnp.int32, (HP, D), 0)
        wo_p = jnp.concatenate(
            [jnp.where((wrow < DH) if h % 2 == 0 else (wrow >= PAD),
                       wo[win(h):win(h) + HP], 0.0) for h in range(H)], axis=0)
        wot_s[...] = _pk(_up(_zip16(wo_p)).T)
        b2c_s[...] = jnp.broadcast_to(b2_ref[...].astype(f32).reshape(1, D), (128, D)).T

    def proj_store(c0, gi, y):
        n = y.shape[1]
        cols = pl.ds(c0, n)
        kind, g = divmod(gi, NG)
        if kind == 0:
            qg = y * qscale
            for i in range(HG):
                lo, hi = qwin(i)
                grow = jax.lax.broadcasted_iota(jnp.int32, (hi - lo, n), 0)
                msk = (grow >= i * DH - lo) & (grow < (i + 1) * DH - lo)
                qm = jnp.where(msk, qg[lo:hi], 0.0).astype(bf16)
                qt_s[g * HG + i, lo // 2:hi // 2, cols] = _pk(qm)
                qf_s[g * HG + i, :, cols] = qg[win(i):win(i) + HP]
        elif kind == 1:
            if c0 + n == S:
                for i in range(HG):
                    kf_s[g * HG + i] = y[win(i):win(i) + HP, n - KV:n]
            k_s[g, pl.ds(c0 // 2, n // 2), :] = _pk(
                jnp.concatenate([y, jnp.zeros((128 - GW, n), f32)], axis=0).astype(bf16).T)
        else:
            hrow = jax.lax.broadcasted_iota(jnp.int32, (HP, n), 0)
            for i in range(HG):
                vw = y[win(i):win(i) + HP]
                if i % 2 == 0:
                    vw = jnp.where(hrow < DH, vw, jnp.where(hrow == DH, 1.0, 0.0))
                else:
                    vw = jnp.where(hrow >= PAD, vw, jnp.where(hrow == 0, 1.0, 0.0))
                vt_s[g * HG + i, :, cols] = _pk(vw.astype(bf16))

    HT = TR // 2
    NT = TR // 128
    KA, KB = 256, D - 256
    SHORT = (3, 4, 6)
    GH = GW // 2

    def pair_rows(p):
        g = (p // 2) * NG + p % 2
        return g, g + NG // 2

    def wsum_steps():
        for p in range(3 * NG // 2):
            for a in range(0, GH, 8):
                v = yield
                wt_s[3 * D // 2:3 * D // 2 + 8, 0:128] = pltpu.bitcast(v[0:8, 0:128], u32)
                blks = []
                for g in pair_rows(p):
                    w = wt_s[pl.ds(pl.multiple_of(o + (g * GH + a), 8), 8), :]
                    blks += [_unzip(w[:, :KA]), _unzip(jnp.concatenate(
                        [w[:, KA:], jnp.zeros((8, KA - KB), u32)], axis=1))]
                for i, op in enumerate(_lhs_ops(*blks)):
                    if i not in (2, 3):
                        aq_s[i - 2 * (i > 3), p * GH + a:p * GH + a + 8, :] = _zip(op[:8], op[8:])
        while True:
            yield

    def xtile(r, rows, t):
        return xt_ref[rows[0]:rows[1], r * TR + t * 128:r * TR + (t + 1) * 128].astype(f32)

    def xform_steps(r, k, n):
        st = []
        for t in range(NT):
            z = after((yield))
            st.append(_stats_t(xtile(r, (0, D), t), k, z))
        for _ in range(XGAP):
            yield
        q = 0
        for t in range(NT // 2):
            for a in range(0, KA, 16):
                if q % n == 0:
                    z = after((yield))
                q += 1
                blks = []
                for i in range(2):
                    for tt in (t, t + NT // 2):
                        if i * KA + a < D:
                            mu = st[tt][0] + z
                            x = xtile(r, (i * KA + a, i * KA + a + 16), tt)
                            blks.append((x - jnp.concatenate([mu, mu], axis=0)) * st[tt][1])
                if a < KB:
                    ops = _rhs_ops(*blks)
                else:
                    ops = [blks[0], blks[0], blks[1], None, None, blks[0] + blks[1], None]
                for i, op in enumerate(ops):
                    if op is not None:
                        t_s[r % 2][0, i, a // 2:a // 2 + 8, t * 128:(t + 1) * 128] = _zip(op[:8], op[8:])
        while True:
            yield

    def kb_gen(src, dst, st, nst, rel):
        n = HB * KV // 128 * DH
        for e in range(n)[n * st // nst:n * (st + 1) // nst]:
            b, t, d = e // (n // HB), e % (n // HB) // DH, e % DH
            row = kf_s[src(b), pl.ds(PAD * (b % 2) + d, 1), t * 128:(t + 1) * 128]
            row = jnp.broadcast_to(row, (8, 128)) + after(rel)
            kt = jnp.concatenate([row] * 16, axis=0).T
            for i in range(16):
                p = t * 16 + i - (KV // 8 - NP)
                if p >= 0:
                    kb_s[dst(b), p, d] = kt[i * 8:(i + 1) * 8]

    def qk_vpu(hk, hq, u, p, par, chain=None, lag=0):
        j, off = u % NJ, PAD * ((u // NJ) % 2)
        acc = None
        for d in range(DH):
            kb = kb_s[hk, NP - 1 - p, d]
            if chain is not None and len(chain) >= lag:
                i = d % (TQ // 128) * 128
                kb = jnp.where(z_s[0:8, 0:128] != 0.0, chain[-lag][:, i:i + 128], kb)
            t = jnp.concatenate(
                [kb * qf_s[hq, pl.ds(off + d, 1), pl.ds(j * TQ + i * 128, 128)]
                 for i in range(TQ // 128)], axis=1)
            acc = t if acc is None else acc + t
            if chain is not None:
                chain.append(acc)
        if p < NPS[u]:
            sv_s[u][par, pl.ds(8 * (NPS[u] - 1 - p), 8), :] = acc
        else:
            s_s[u, pl.ds(S - 8 * p - 8, 8), :] = acc
        return acc

    def gated(x, gates):
        if not gates:
            return x
        parts = [x[i:i + 8] for i in range(0, x.shape[0], 8)]
        never = z_s[0:8, 0:128] != 0.0
        for g, r in gates:
            y = jnp.where(never, pltpu.bitcast(g, u32), parts[r][:, 0:128])
            parts[r] = jnp.concatenate([y, parts[r][:, 128:]], axis=1) if x.shape[1] > 128 else y
        return jnp.concatenate(parts, axis=0)

    first = dict(n=0, chain=[])
    mx = {}

    def col_max(u, m):
        if u in mx:
            m_s[u] = jnp.max(jnp.maximum(m, mp_s[o + u]), axis=0, keepdims=True)
        else:
            mx[u] = mp_s[u] = m

    def first_step(r, rel):
        n, ov, gates = first["n"], first["ov"], []
        first["n"] += 1
        if rel is not None:
            kb_gen(lambda b: b, lambda b: H - HB + b, n, GSA[0], rel)
            if n >= GSA[0]:
                kb_gen(lambda b: HB + b, lambda b: ov + b, n - GSA[0], GSA[1], rel)
        for us, (e0, e1), lag in zip(UORD, EV, CHN):
            seq = [(u, p) for u in us for p in range(NPB[u])]
            lo, hi = [max(len(seq) * (e - e0) // (e1 - e0), 0) for e in (n, n + 1)]
            for u, p in seq[lo:hi]:
                v = qk_vpu(ov + (H - HB + u // NJ), u // NJ, u, p, 0, first["chain"], lag)
                first["m"] = jnp.maximum(first["m"], v) if p else v
                if p + 1 == NPB[u]:
                    col_max(u, first["m"])
                gates += [(v[:, i:i + 128], r) for i in range(0, TQ, 128)]
        return gates

    def started(gen):
        next(gen)
        return gen

    wsum = started(wsum_steps())
    xform = started(xform_steps(0, K11, XN1))
    for n, g0 in enumerate(GORDER):
        g1 = g0 + (2 if n == 0 else 1)
        n = n + 1 if n else 0
        if n == G_WB:
            copies["wb"].wait()
            wt_prep(WA, WB)
        if n == G_WC:
            copies["wc"].wait()
            copies["x1"].wait()
            wt_prep(WB, 3 * D)
        y = jnp.dot(_up(wt_s[g0 * GH:g1 * GH, :]), xn0, preferred_element_type=f32)
        for gi in range(g0, g1):
            proj_store(S - TR, gi, y[(gi - g0) * GW:(gi - g0 + 1) * GW])
        for t in range(NT):
            if n >= G_WS:
                for a in WSROWS:
                    wsum.send(y[a:a + 8, t * 128:(t + 1) * 128])
            if n >= G_X1:
                xform.send(y[56:64, t * 128:(t + 1) * 128])
    for r in range(NR - 1):
        xform = started(xform_steps(r + 1, K1, XN)) if r + 2 < NR else None

        def tick(v):
            wsum.send(v)
            if r > 0 or p >= P_X2:
                first["gates"] = first_step(GA, v)
            if xform is not None and (r > 0 or p >= P_X2):
                xform.send(v)

        for p in range(3 * NG // 2):
            if r == 0 and p == P_X2:
                copies["x2"].wait()
                first["ov"] = jax.lax.rem(o_s[0], 7)
            ms = [m.at[:, 0:GW] for m in ms_s[p % NMS * 9:][:5]]
            gs = pair_rows(p)

            def mm(i):
                kk = KB if i in SHORT else KA
                if i == 2:
                    w = wt_s[gs[0] * GH:(gs[0] + 1) * GH, 0:KA]
                elif i == 3:
                    w = wt_s[gs[1] * GH:(gs[1] + 1) * GH, KA:D]
                else:
                    w = aq_s[i - 2 * (i > 3), p * GH:(p + 1) * GH, 0:kk]
                w = gated(w, first.pop("gates", None))
                return jnp.dot(_up(w), _up(t_s[r % 2][o, i, 0:kk // 2, :]),
                               preferred_element_type=f32)

            m = mm(0); ms[0][0] = m; tick(m)
            m = mm(2); ms[2][0] = m; tick(m)
            m = mm(1); ms[1][0] = m; tick(m)
            m = mm(4); ms[4][0] = m; proj_store(r * TR + HT, gs[0], m + ms[2][o]); tick(m)
            m = mm(3); ms[3][0] = m; proj_store(r * TR, gs[1], m + ms[1][o]); tick(m)
            m = mm(5)
            proj_store(r * TR + HT, gs[1], ((m + ms[0][o]) + ms[2][o]) - ms[1][o]); tick(m)
            m = mm(6)
            proj_store(r * TR, gs[0], ((m + ms[0][o]) + ms[3][o]) - ms[4][o]); tick(m)

    def qk_rows(h, u, a, b, par, m, gates):
        j = u % NJ
        qt = _up(qt_s[h, :, pl.ds(j * TQ, TQ)])
        k = k_s[h // HG, a // 2:b // 2, :]
        s = jnp.dot(_up(gated(k, gates)), qt, preferred_element_type=f32)
        SM = SMS[u]
        if a < SM:
            s_s[u, a:min(b, SM), :] = s[:min(b, SM) - a]
        if b > SM:
            sv_s[u][par, max(a, SM) - SM:b - SM, :] = s[max(a, SM) - a:]
        mc = jnp.max(s.reshape((b - a) // 8, 8, TQ), axis=0)
        return mc if m is None else jnp.maximum(m, mc)

    def qk_step(h, hk, hq, u, c, n, nc, par, m):
        vs = [qk_vpu(hk, hq, u, p, par)
              for p in range(n)[::-1][n * c // nc:n * (c + 1) // nc]]
        gates = [(v[:, i:i + 128], GR) for v in vs for i in range(0, TQ, 128)]
        a, b = [(S - 8 * n) // 16 * e // NC * 16 for e in (c, c + 1)]
        mv = m[1]
        for v in vs:
            mv = v if mv is None else jnp.maximum(mv, v)
        m = qk_rows(h, u, a, b, par, m[0], gates)
        if c + 1 == NC:
            m_s[u] = jnp.max(m if mv is None else jnp.maximum(m, mv), axis=0, keepdims=True)
        return m, mv

    def pv_chunk(h, u, c, par, m, acc, rel=None):
        lo, hi, SM = c * CK, (c + 1) * CK, SMS[u]
        s = [s_s[u, lo:min(hi, SM), :]] if lo < SM else []
        if hi > SM:
            a = max(lo, SM) - SM
            if rel is not None:
                sv_s[u][1 - par, 8 * NPS[u]:8 * NPS[u] + 8, 0:128] = rel[0:8, 0:128]
                a = pl.multiple_of(o_s[0] + a, 8)
            s.append(sv_s[u][par, pl.ds(a, hi - max(lo, SM)), :])
        p = jnp.exp2(jnp.concatenate(s, axis=0) - m).astype(bf16)
        vt = _up(vt_s[h, :, pl.ds(c * CK, CK)])
        o = jnp.dot(vt, p, preferred_element_type=f32)
        return o if acc is None else acc + o

    def pv_finish(h, u, acc):
        l = acc[DH:DH + 1, :] if (u // NJ) % 2 == 0 else acc[0:1, :]
        r = pl.reciprocal(l, approx=True)
        r = r * (2.0 - l * r)
        ot_s[h, :, pl.ds((u % NJ) * TQ, TQ)] = _zip16(acc * r)

    D2, F2 = D // 2, F // 2

    D4 = D // 4

    def w1_block(t, i, j, v):
        b1 = b1_ref[...].astype(f32)
        arow = jax.lax.broadcasted_iota(jnp.int32, (DA, 128), 0)
        tt = i * (NF // 2) + t
        aug = jnp.where(arow == 2 * i + j, b1[tt:tt + 1, :], 0.0).astype(bf16)
        w1_ref[D:D + 16, 0:128] = pltpu.bitcast(v[0:8, 0:128], bf16)
        w = w1_ref[pl.ds(pl.multiple_of(o + j * D2, 16), D2), tt * 128:(tt + 1) * 128].astype(f32)
        w = jnp.concatenate([_up(_zip(w[:D4], w[D4:])), aug], axis=0)
        w1t_s[j, tt * 64:(tt + 1) * 64, :] = _pk(_unzip(_pk(w.T)).astype(bf16))

    def w1_sums(a, v):
        w1t_s[0, F2:F2 + 8, 0:128] = pltpu.bitcast(v[0:8, 0:128], u32)
        blks = [_unzip(w1t_s[j, pl.ds(pl.multiple_of(o + (i * (F2 // 2) + a), 8), 8), :])
                for i in range(2) for j in range(2)]
        for i, op in enumerate(_lhs_ops(*blks)):
            if i not in (2, 3):
                out = a1_s[i - 2 * (i > 3), a:a + 8, :] = _zip(op[:8], op[8:])
        return out[:, 0:128]

    def w2_steps():
        for q in range(NF // 2):
            for a in range(0, D2, W2S):
                v = yield
                w2t_ref[D:D + 16, 0:128] = pltpu.bitcast(v[0:8, 0:128], bf16)
                blks = [_unzip(_pk(w2t_ref[pl.ds(pl.multiple_of(o + (i * D2 + a), W2S), W2S),
                                           j * F2 + q * 128:j * F2 + (q + 1) * 128]))
                        for i in range(2) for j in range(2)]
                for i, op in enumerate(_lhs_ops(*blks)):
                    a2_s[i, a // 2:(a + W2S) // 2, q * 128:(q + 1) * 128] = _zip(
                        op[:W2S // 2], op[W2S // 2:])
        while True:
            yield

    w2sum = started(w2_steps())
    due = {}
    for u in range(HB * NJ):
        if u == 1:
            for n in ("b1", "b2", "wo", "w1", "w2"):
                copies[n].wait()
            first.update(ov=jax.lax.rem(o_s[0], 7), chain=[])
            prep_small()
            xrow = jax.lax.broadcasted_iota(jnp.int32, (DA, TR // 2), 0)
            xaug = _pk(jnp.where(xrow < 4, 1.0, 0.0).astype(bf16))
            for t in t_s:
                for i in BIASED:
                    t[0, i, D4:D4 + DA // 2, :] = xaug
        m = None
        for c in range(NC):
            gates = first.pop("gates", [])
            if u >= 1 and c == WG:
                gates.append((w1t_s[0, pl.ds(pl.multiple_of(o + (u - 1) * 64, 8), 8), 0:128], 0))
            if u * NC + c in due:
                gates.append((due[u * NC + c], 0))
            a, b = [(S - 8 * NPB[u]) // 16 * e // NC * 16 for e in (c, c + 1)]
            m = qk_rows(u // NJ, u, a, b, 0, m, gates)
            if c + 1 == NC:
                col_max(u, m)
            first["gates"] = first_step(GR, m if u == 0 else None)
            if u >= 1:
                if c < 4:
                    w1_block(u - 1, c // 2, c % 2, m)
                if c in W2C:
                    w2sum.send(m)
                for k in range(8):
                    if c == WG + k * (NC - WG) // 8:
                        due[u * NC + c + WD] = w1_sums((u - 1) * 64 + k * 8, m)

    NIT = H // HB - 1

    def body(it, carry):
        par = it % 2
        itv = jax.lax.rem(it, NIT)
        pending = None
        for u in range(HB * NJ):
            h = it * HB + u // NJ
            mcur = m_s[u]
            hv = itv * HB + u // NJ
            hist = [(None, None)]
            acc = z_s[...] if u > 0 else None
            for c in range(NC):
                acc = pv_chunk(h, u, c, par, mcur, acc, hist[max(c + 1 - RL, 0)][0])
                hist.append(qk_step(h + HB, hv, hv + HB, u, c, NPS[u], NCV, 1 - par, hist[-1]))
                kb_gen(lambda b: itv * HB + (2 * HB + b), lambda b: itv * HB + (HB + b),
                       u * NC + c, GS, hist[-1][0])
                if c == DEFER and pending is not None:
                    pv_finish(*pending)
            pending = (h, u, acc)
        pv_finish(*pending)
        return carry

    jax.lax.fori_loop(0, NIT, body, 0)

    o = o_s[0]
    z_s[0:8, 0:128] = after(kb_s[o, 0, 0])
    HE = H - HG

    def pv_steps(r):
        pending = None
        for b in range(HB):
            u = b * NJ + r
            h = H - HB + b
            mcur = m_s[u]
            acc = z_s[...]
            for c in range(NC):
                acc = pv_chunk(h, u, c, NIT % 2, mcur, acc)
                if c == DEFER and pending is not None:
                    pv_finish(*pending)
                if b == HB - 1 and c == NC - 1:
                    pv_finish(h, u, acc)
                yield
            pending = (h, u, acc)

    def advance(gen, n):
        v = None
        for _ in range(n):
            v = next(gen, None)
        return v

    def oproj(r, rows, h0, h1):
        cols = pl.ds(r * TR, TR)
        ot = _up(ot_s[h0:h1, :, cols].reshape((h1 - h0) * HP // 2, TR))
        w = _up(wot_s[rows[0] // 2:rows[1] // 2, h0 * HP:h1 * HP])
        return jnp.dot(w, ot, preferred_element_type=f32)

    def part(r, rows, h1=HE):
        return (xt_ref[rows[0]:rows[1], pl.ds(r * TR, TR)].astype(f32)
                + oproj(r, rows, 0, h1))

    def stats2(h1, t, k, dep):
        return _stats_t(h1[:, t * 128:(t + 1) * 128], k, None if dep is None else after(dep))

    def form_steps(r, h1, st, n):
        z = None
        for t in range(NT // 2):
            for q, a in enumerate(range(0, D4, 8)):
                if (t * (D4 // 8) + q) % n == 0:
                    z = after((yield))
                blks = []
                for i in range(2):
                    for tt in (t, t + NT // 2):
                        x = jnp.concatenate(
                            [h1[i * D2 + e * D4 + a:i * D2 + e * D4 + a + 8, tt * 128:(tt + 1) * 128]
                             for e in range(2)], axis=0)
                        mu = st[tt][0] + z
                        blks.append((x - jnp.concatenate([mu, mu], axis=0)) * st[tt][1])
                for i, op in enumerate(_rhs_ops(*blks)):
                    t_s[r % 2][0, i, a:a + 8, t * 128:(t + 1) * 128] = _zip(op[:8], op[8:])
        while True:
            yield

    def part_steps(r, out):
        for a in range(0, D, PR):
            rows = (a, min(a + PR, D))
            acc = xt_ref[rows[0]:rows[1], pl.ds(r * TR, TR)].astype(f32)
            for g in range(HE // HG):
                acc = acc + oproj(r, rows, g * HG, (g + 1) * HG)
                if g == HE // HG - 1:
                    out.append(acc)
                yield acc

    def strassen(mm, tick, fin):
        m3 = mm(2); tick(m3)
        m5 = mm(4)
        fin(0, 1, m5 + m3); tick(m5)
        m2 = mm(1); tick(m2)
        m4 = mm(3)
        fin(1, 0, m4 + m2); tick(m4)
        m1 = mm(0); tick(m1)
        m7 = mm(6)
        fin(0, 0, ((m7 + m1) + m4) - m5); tick(m7)
        m6 = mm(5)
        fin(1, 1, ((m6 + m1) + m3) - m2); tick(m6)

    gen = pv_steps(0)
    parts = [[] for _ in range(3)]
    fill = (x for r in range(3) for x in part_steps(r, parts[r]))
    for q in range(HB * NC):
        advance(fill, 1)
        advance(gen, 1)
    advance(fill, FILL)
    h1 = jnp.concatenate(parts[0], axis=0) + oproj(0, (0, D), HE, H)
    st = [stats2(h1, 0, K20, None)]
    for t in range(1, NT):
        st.append(stats2(h1, t, K20, advance(fill, FILL2[t - 1])))
    advance(fill, FILL3)
    form = form_steps(0, h1, st, FORMN0)
    next(form)
    for v in fill:
        form.send(v)
    for r in range(NR):
        gen = pv_steps(r + 1) if r + 1 < NR else iter(())
        h1cur = h1
        st = []
        state = dict(n=0)

        def tick(v):
            state["n"] += 1
            n = state["n"]
            advance(gen, 1)
            if r + 1 < NR:
                if n == OPD:
                    if r + 1 < len(parts):
                        state["h1"] = (jnp.concatenate(parts[r + 1], axis=0)
                                       + oproj(r + 1, (0, D), HE, H))
                    else:
                        state["h1"] = part(r + 1, (0, D), H)
                if n in LNT:
                    st.append(stats2(state["h1"], len(st), K2, v))
                if n == FORM0:
                    state["form"] = form_steps(r + 1, state["h1"], st, FORMN)
                    next(state["form"])
                if n >= FORM0:
                    state["form"].send(v)

        def act(c):
            c = jnp.maximum(c, 0.0)
            return c * c

        late = [lambda: None] * 2
        for a in range(0, F2, FQ):
            ms = ms_s[(a // FQ) % NMS * 9:][:9]
            rows = slice(a // 2, (a + FQ) // 2)

            def mm(i):
                kk = D2 + DA if i in BIASED else D2
                if i in (2, 3):
                    w = w1t_s[i - 2, pl.ds((i - 2) * F2 // 2 + a // 2, FQ // 2), 0:kk]
                else:
                    w = a1_s[i - 2 * (i > 3), rows, 0:kk]
                return jnp.dot(_up(w), _up(t_s[r % 2][o, i, 0:kk // 2, :]),
                               preferred_element_type=f32)

            def put(i, v, p=a // FQ):
                v = _zip(v[:FQ // 2], v[FQ // 2:])
                if (p + 1) * FQ < F2:
                    u_s[0, i, p * FQ // 2:(p + 1) * FQ // 2, :] = v
                else:
                    ul_s[i][0] = v

            m = mm(0); ms[0][0] = m; late.pop(0)(); tick(m)
            m = mm(2); ms[2][0] = m; late.pop(0)(); tick(m)
            m = mm(1); ms[1][0] = m; tick(m)
            m = mm(4); ms[4][0] = m; ms[6][0] = act(m + ms[2][o]); tick(m)
            m = mm(3); ms[3][0] = m; ms[7][0] = act(m + ms[1][o]); tick(m)
            m = mm(5)
            b = act(((m + ms[0][o]) + ms[2][o]) - ms[1][o])
            ms[8][0] = b
            put(4, b); put(2, ms[6][o] - b); tick(m)
            m = mm(6)
            b = act(((m + ms[0][o]) + ms[3][o]) - ms[4][o])
            ms[5][0] = b
            put(1, b); put(3, ms[7][o] - b); put(5, b + ms[6][o]); tick(m)
            late = [lambda ms=ms, put=put: put(6, ms[7][o] + ms[8][o]),
                    lambda ms=ms, put=put: put(0, ms[5][o] + ms[8][o])]
        for f in late:
            f()
        split = F2LAST if r + 1 == NR else F2SPLIT
        for a, b in zip(split[:-1], split[1:]):
            last = r + 1 == NR and b == D2

            def fin2(i, j, c):
                rows = slice(i * D2 + a, i * D2 + b)
                cols = pl.ds(r * TR + j * HT, HT)
                b2c = jnp.concatenate([b2c_s[rows]] * (HT // 128), axis=1)
                out_ref[rows, cols] = (h1cur[rows, j * HT:(j + 1) * HT] + c + b2c).astype(out_ref.dtype)
                if r + 1 == NR and i == j:
                    out_copy(pl.ds(i * D2 + a, b - a), pl.ds(r * TR, TR)).start()

            strassen(lambda i: jnp.dot(_up(a2_s[i, a // 2:b // 2, :]), _up(jnp.concatenate([u_s[o, i], ul_s[i][o]], axis=0)),
                                       preferred_element_type=f32), tick, fin2)
        if r + 1 < NR:
            out_copy(pl.ds(0, D), pl.ds(r * TR, TR)).start()
            h1 = state["h1"]
    for cp in out_copies:
        cp.wait()


@jax.jit
def pallas_sequential_preLN__softmax_full_mha__dense_activation_squared_relu__prompt_kernel(
    A_x: jax.Array,
    A_wqkv: jax.Array,
    A_wo: jax.Array,
    B_x: jax.Array,
    B_w1: jax.Array,
    B_b1: jax.Array,
    B_w2: jax.Array,
    B_b2: jax.Array,
):
    del B_x
    B, S, D = A_x.shape
    F = B_w1.shape[1]
    assert B == 1 and TR == TQ
    out_t = pl.pallas_call(
        _kernel,
        out_shape=jax.ShapeDtypeStruct((D, S), A_x.dtype),
        in_specs=[pl.BlockSpec(memory_space=pl.ANY)] * 7,
        out_specs=pl.BlockSpec(memory_space=pl.ANY),
        scratch_shapes=[
            pltpu.VMEM((D, S), bf16),
            pltpu.VMEM((D, 3 * D), bf16),
            pltpu.VMEM((D, D), bf16),
            pltpu.VMEM((D + 32, F), bf16),
            pltpu.VMEM((D + 32, F), bf16),
            pltpu.VMEM((D, S), bf16),
            pltpu.VMEM((3 * D // 2 + 8, D), u32),
            pltpu.VMEM((5, 3 * D // 4, 256), u32),
            pltpu.VMEM((D // 2, H * HP), u32),
            pltpu.VMEM((2, F // 2 + 16, D // 2 + DA), u32),
            pltpu.VMEM((5, F // 4, D // 2 + DA), u32),
            pltpu.VMEM((D, 128), f32),
            pltpu.VMEM((H // HG, S // 2, 128), u32),
            pltpu.VMEM((H, 64, S), u32),
            pltpu.VMEM((H, HP // 2, S), u32),
            pltpu.VMEM((H, HP // 2, S), u32),
            pltpu.VMEM((HB * S // TQ, S - 8 * min(NPS), TQ), f32),
            [pltpu.VMEM((2, 8 * n + 8, TQ), f32) for n in NPS],
            pltpu.VMEM((H, HP, S), f32),
            pltpu.VMEM((H + HB, HP, -(-NP // 16) * 128), f32),
            pltpu.VMEM((H, NP, D // H, 8, 128), f32),
            pltpu.VMEM((HP, TQ), f32),
            pltpu.VMEM((HB * S // TQ, 8, TQ), f32),
            pltpu.VMEM((HB * S // TQ, 1, TQ), f32),
            [pltpu.VMEM((1, FQ, TR // 2), f32)] * (9 * NMS),
            pltpu.VMEM((1, 7, F // 4 - FQ // 2, TR // 2), u32),
            [pltpu.VMEM((1, FQ // 2, TR // 2), u32)] * 7,
            [pltpu.VMEM((1, 7, 128, TR // 2), u32)] * 2,
            pltpu.VMEM((7, D // 4, F // 2), u32),
            pltpu.VMEM((F // 128, 128), bf16),
            pltpu.VMEM((D,), bf16),
            pltpu.SMEM((1,), jnp.int32),
            pltpu.SemaphoreType.DMA((6,)),
        ],
        compiler_params=pltpu.CompilerParams(vmem_limit_bytes=124 * 2**20),
    )(A_x.reshape(S, D).T, A_wqkv, A_wo, B_w1, B_b1.reshape(F // 128, 128), B_w2.T,
      B_b2)
    return out_t.T.reshape(B, S, D)
```
